```python
import jax
import jax.numpy as jnp

def _softmax(x, axis=-1):
    return jax.nn.softmax(x, axis=axis)

def _gelu(x):
    return jax.nn.gelu(x, approximate=True)

def _silu(x):
    return jax.nn.silu(x)

def _sigmoid(x):
    return jax.nn.sigmoid(x)

def _layernorm(x, axis=-1, eps=1e-05):
    m = jnp.mean(x, axis=axis, keepdims=True)
    v = jnp.var(x, axis=axis, keepdims=True)
    return (x - m) / jnp.sqrt(v + eps)

def _scatter_add(tgt, idx, src, axis=0):
    return tgt.at[idx].add(src)

def _segment_sum(src, seg, n):
    return jax.ops.segment_sum(src, seg, n)

class _Rng:

    def __init__(self, key):
        self._k = key

    def _next(self):
        self._k, sub = jax.random.split(self._k)
        return sub

    def normal(self, shape):
        return jax.random.normal(self._next(), shape, dtype=jnp.bfloat16)

    def randint(self, lo, hi, shape):
        return jax.random.randint(self._next(), shape, lo, hi, dtype=jnp.int32)

    def uniform(self, shape, lo=0.0, hi=1.0):
        return jax.random.uniform(self._next(), shape, jnp.bfloat16, lo, hi)

    def permutation(self, n):
        return jax.random.permutation(self._next(), n)
kernel_name = 'gated_mix__ssm_conv_h3__memory_aug_recurrent_mem_tr__prompt'

def setup_inputs():
    _rng = _Rng(jax.random.key(int.from_bytes(__import__("os").urandom(4), "little")))
    _w = lambda a: (lambda t: t.astype(jnp.bfloat16) if jnp.issubdtype(t.dtype, jnp.floating) else t)(jnp.asarray(a))

    def _A_setup():
        B, S, D = (1, 2048, 1024)
        ks = 4
        return {'q': _w((lambda *s: _rng.normal(s) * 0.05)(B, S, D)), 'k': _w((lambda *s: _rng.normal(s) * 0.05)(B, S, D)), 'v': _w((lambda *s: _rng.normal(s) * 0.05)(B, S, D)), 'shift_k': _w((lambda *s: _rng.normal(s) * 0.05)(D, ks) * 0.5), 'ssm_k': _w((lambda *s: _rng.normal(s) * 0.05)(D, S) * (1.0 / S ** 0.5)), 'ssm_D': _w((lambda *s: _rng.normal(s) * 0.05)(D))}
    _A_in = _A_setup()

    def _B_setup():
        B, S, Dm = (1, 2048, 1024)
        H, Dh = (32, 128)
        M, seg = (8, 32)
        seg = min(seg, S)
        S = S // seg * seg
        return {'x': _w((lambda *s: _rng.normal(s) * 0.05)(B, S, Dm)), 'mem0': _w((lambda *s: _rng.normal(s) * 0.05)(B, M, Dm)), 'Wq': _w((lambda *s: _rng.normal(s) * 0.05)(Dm, H, Dh) * Dm ** (-0.5)), 'Wk': _w((lambda *s: _rng.normal(s) * 0.05)(Dm, H, Dh) * Dm ** (-0.5)), 'Wv': _w((lambda *s: _rng.normal(s) * 0.05)(Dm, H, Dh) * Dm ** (-0.5)), 'Wo': _w((lambda *s: _rng.normal(s) * 0.05)(H, Dh, Dm) * (H * Dh) ** (-0.5)), 'seg_len': seg}
    _B_in = _B_setup()
    return {'A_q': _A_in['q'], 'A_k': _A_in['k'], 'A_v': _A_in['v'], 'A_shift_k': _A_in['shift_k'], 'A_ssm_k': _A_in['ssm_k'], 'A_ssm_D': _A_in['ssm_D'], 'B_x': _B_in['x'], 'B_mem0': _B_in['mem0'], 'B_Wq': _B_in['Wq'], 'B_Wk': _B_in['Wk'], 'B_Wv': _B_in['Wv'], 'B_Wo': _B_in['Wo'], 'B_seg_len': _B_in['seg_len'], 'gate_w': _w((lambda *s: _rng.normal(s) * 0.05)(1024))}

def reference(A_q, A_k, A_v, A_shift_k, A_ssm_k, A_ssm_D, B_x, B_mem0, B_Wq, B_Wk, B_Wv, B_Wo, B_seg_len, gate_w):

    def _A_ref(q, k, v, shift_k, ssm_k, ssm_D):
        B, S, D = q.shape
        ks = shift_k.shape[-1]
        k_pad = jnp.pad(k, ((0, 0), (ks - 1, 0), (0, 0)))
        k_shift = jnp.zeros_like(k)
        for t in range(ks):
            k_shift = k_shift + k_pad[:, t:t + S, :] * shift_k[:, ks - 1 - t][None, None, :]
        kv = k_shift * v
        L = 2 * S
        kv_pad = jnp.pad(kv, ((0, 0), (0, S), (0, 0)))
        kf_pad = jnp.pad(ssm_k, ((0, 0), (0, S)))
        kv_f = (lambda x, axes=(-2, -1): jnp.fft.rfft2(x.astype(jnp.float32), axes=axes))(kv_pad[:, None, :, :], axes=(1, 2))
        kf_f = (lambda x, axes=(-2, -1): jnp.fft.rfft2(x.astype(jnp.float32), axes=axes))(kf_pad[:, None, :], axes=(1, 2))
        kf_f = (lambda x, *d: x.transpose(*d))(kf_f, 1, 2, 0)
        y_f = kv_f * kf_f[None, :, :, :]
        y = (lambda x, s, axes=(-2, -1): jnp.fft.irfft2(x, s=s, axes=axes).astype(jnp.bfloat16))(y_f, (1, L), axes=(1, 2))[:, 0, :S, :]
        y = y + kv * ssm_D[None, None, :]
        return q * y

    def _B_ref(x, mem0, Wq, Wk, Wv, Wo, seg_len):
        B, S, Dm = x.shape
        H, Dh = (Wq.shape[1], Wq.shape[2])
        M = mem0.shape[1]
        scale = Dh ** (-0.5)
        n_seg = S // seg_len
        L = M + seg_len
        idx = jnp.arange(L)
        mask = (idx[:, None] < M) | (idx[:, None] >= idx[None, :])
        mem = mem0
        outs = []
        for s in range(n_seg):
            xs = x[:, s * seg_len:(s + 1) * seg_len, :].copy()
            h = jnp.concatenate([mem, xs], axis=1)
            q = jnp.einsum('btd,dhe->bhte', h, Wq)
            k = jnp.einsum('btd,dhe->bhte', h, Wk)
            v = jnp.einsum('btd,dhe->bhte', h, Wv)
            scores = jnp.einsum('bhqe,bhke->bhqk', q, k) * scale
            scores = jnp.where(mask[None, None], scores, -1000000000.0)
            p = _softmax(scores, axis=-1)
            o = jnp.einsum('bhqk,bhke->bhqe', p, v)
            o = jnp.einsum('bhte,hed->btd', o, Wo)
            mem = o[:, :M, :].copy()
            outs.append(o[:, M:, :])
        return jnp.concatenate(outs, axis=1)
    x = A_q
    g = _sigmoid((x * gate_w).sum(-1, keepdims=True))
    a = _A_ref(x, A_k, A_v, A_shift_k, A_ssm_k, A_ssm_D)
    b = _B_ref(x, B_mem0, B_Wq, B_Wk, B_Wv, B_Wo, B_seg_len)
    return g * a + (1 - g) * b
```

```python
import functools

import jax
import jax.numpy as jnp
import ml_dtypes
import numpy as np
from jax.experimental import pallas as pl
from jax.experimental.pallas import tpu as pltpu

S, D, H, DH, M, SEG = 2048, 1024, 32, 128, 8, 32
NT = D // 128
NBLK = S // (2 * SEG)
CH = 128
F32, BF16 = jnp.float32, jnp.bfloat16


def _make_consts():
    n, tp = 2 * S, 2 * np.pi
    t1 = np.arange(16)
    c1 = np.zeros((16, 256, 128))
    c1i = np.zeros((16, 128, 256))
    for g in range(16):
        for s in range(8):
            t = 128 * t1 + 8 * g + s
            cols = t1 * 8 + s
            c1[g, s, cols] = 1.0
            c1[g, 8 + s, cols] = (-1.0) ** t1
            c1i[g, cols, s] = 1.0 / n
            c1i[g, cols, 8 + s] = (-1.0) ** t1 / n
            for j in range(1, 16):
                ph = tp * ((t * j) % n) / n
                c1[g, 16 * j + s, cols] = np.cos(ph)
                c1[g, 16 * j + 8 + s, cols] = -np.sin(ph)
                c1i[g, cols, 16 * j + s] = 2 * np.cos(ph) / n
                c1i[g, cols, 16 * j + 8 + s] = -2 * np.sin(ph) / n
    a = np.arange(128)
    th = tp * ((a[:, None] * a[None, :]) % 128) / 128
    c, s_ = np.cos(th), np.sin(th)
    th16 = tp * ((a[None, :] * (32 * a[:, None] + 16)) % n) / n
    c2 = np.block([[c, s_], [-s_, c]])
    c2i = np.block([[c, -s_], [s_, c]])
    c2e = np.stack([np.concatenate([c, -s_], 0),
                    np.concatenate([np.cos(th16), -np.sin(th16)], 0)])
    c2ie = np.stack([np.concatenate([c, -s_], 1),
                     np.concatenate([np.cos(th16.T), -np.sin(th16.T)], 1)])
    return tuple(x.astype(ml_dtypes.bfloat16) for x in (c1, c1i, c2, c2i, c2e, c2ie))


_CONSTS = _make_consts()


def _dot(a, b):
    return jnp.dot(a, b, preferred_element_type=F32)


def _kernel(x_hbm, k_hbm, v_hbm, f_hbm, wq_hbm, wk_hbm, wv_hbm, wo_hbm,
            shift_ref, ssmd_ref, gate_ref, mem0_ref,
            c1_ref, c1i_ref, c2_ref, c2i_ref, c2e_ref, c2ie_ref,
            out_hbm,
            xs, xf, ab, ks, vs, fs, wst, wqkv, wo_v, kpad, sig, yb, ub, gbuf, carry, ob,
            sem_x, sem_a, sem_w, sem_wo, sem_o):
    w_hbm = (wq_hbm, wk_hbm, wv_hbm)

    def x_copy(n):
        return pltpu.make_async_copy(x_hbm.at[0, :, pl.ds(n * 128, 128)], xs.at[n], sem_x.at[n])

    def wo_copy(n):
        return pltpu.make_async_copy(wo_hbm.at[:, :, pl.ds(n * 128, 128)], wo_v.at[n], sem_wo.at[n])

    def a_copies(dt, slot):
        c0 = pl.multiple_of(dt * 128, 128)
        return (pltpu.make_async_copy(k_hbm.at[0, :, pl.ds(c0, 128)], ks.at[slot], sem_a.at[0, slot]),
                pltpu.make_async_copy(v_hbm.at[0, :, pl.ds(c0, 128)], vs.at[slot], sem_a.at[1, slot]),
                pltpu.make_async_copy(f_hbm.at[pl.ds(c0, 128), :], fs.at[slot], sem_a.at[2, slot]))

    def w_copies(c, slot):
        r0 = pl.multiple_of(c * CH, CH)
        return tuple(pltpu.make_async_copy(w_hbm[m].at[pl.ds(r0, CH)], wst.at[slot, m], sem_w.at[m, slot])
                     for m in range(3))

    for cp in a_copies(0, 0):
        cp.start()
    x_copy(0).start()
    for cp in w_copies(0, 0):
        cp.start()
    for n in range(1, NT):
        x_copy(n).start()
    for n in range(NT):
        wo_copy(n).start()
    kpad[0:8, :] = jnp.zeros((8, 128), F32)

    def a_body(dt, _):
        slot = dt % 2
        for cp in a_copies(dt, slot):
            cp.wait()

        @pl.when(dt + 1 < NT)
        def _():
            for cp in a_copies(dt + 1, 1 - slot):
                cp.start()
            for cp in w_copies(dt + 1, 1 - slot):
                cp.start()

        c0 = pl.multiple_of(dt * 128, 128)
        sh = jnp.concatenate([shift_ref[pl.ds(c0, 128), :].astype(F32),
                              jnp.zeros((128, 124), F32)], axis=1).T
        taps = [sh[j:j + 1, :] for j in range(4)]
        dvec = ssmd_ref[dt].astype(F32)
        for b in range(16):
            kpad[8 + b * 128:8 + (b + 1) * 128, :] = ks[slot, b * 128:(b + 1) * 128, :].astype(F32)
        for b in range(16):
            kw = kpad[b * 128:b * 128 + 136, :]
            ksh = kw[8:136] * taps[0]
            for j in range(1, 4):
                ksh = ksh + kw[8 - j:136 - j] * taps[j]
            kv = ksh * vs[slot, b * 128:(b + 1) * 128, :].astype(F32)
            sig[b, :, 0:128] = kv.astype(BF16).astype(F32)
            sig[b, :, 128:256] = fs[slot, :, b * 128:(b + 1) * 128].astype(F32).T
        for g in range(16):
            tile = sig[:, 8 * g:8 * g + 8, :].reshape(128, 256).astype(BF16)
            yb[:, 8 * g:8 * g + 8, :] = _dot(c1_ref[g], tile).reshape(32, 8, 256)

        def cmul(z):
            kr, fr, ki, fi = z[0:128, 0:128], z[0:128, 128:256], z[128:256, 0:128], z[128:256, 128:256]
            return jnp.concatenate([kr * fr - ki * fi, kr * fi + ki * fr], axis=0).astype(BF16)

        for e in range(2):
            z = _dot(c2e_ref[e], yb[e].astype(BF16))
            ub[e] = _dot(c2ie_ref[e], cmul(z))
        for j in range(1, 16):
            z = _dot(c2_ref[...], yb[2 * j:2 * j + 2].reshape(256, 256).astype(BF16))
            ub[2 * j:2 * j + 2] = _dot(c2i_ref[...], cmul(z)).reshape(2, 128, 128)
        x_copy(dt).wait()
        for g in range(16):
            tile = ub[:, 8 * g:8 * g + 8, :].reshape(256, 128).astype(BF16)
            y = _dot(c1i_ref[g], tile).reshape(16, 8, 128)
            kv = sig[:, 8 * g:8 * g + 8, 0:128]
            xq = jnp.stack([xs[dt, b * 128 + 8 * g:b * 128 + 8 * g + 8, :] for b in range(16)]).astype(F32) \
                if False else None
            ab[dt, :, 8 * g:8 * g + 8, :] = y + kv * dvec
        for b in range(16):
            xq = xs[dt, b * 128:(b + 1) * 128, :].astype(F32)
            xf[dt, b] = xq
            ab[dt, b] = ab[dt, b] * xq
        for cp in w_copies(dt, slot):
            cp.wait()
        r0 = dt * (CH // 2)
        for m in range(3):
            for b in range(CH // 16):
                u = pltpu.bitcast(wst[slot, m, b * 16:(b + 1) * 16], jnp.uint32).reshape(8, 2, 16, 128)
                ev, od = u[:, 0], u[:, 1]
                lo = jnp.swapaxes((ev & jnp.uint32(0xFFFF)) | (od << 16), 0, 1)
                hi = jnp.swapaxes((ev >> 16) | (od & jnp.uint32(0xFFFF0000)), 0, 1)
                rows = pl.ds(pl.multiple_of(r0 + b * 8, 8), 8)
                for hp in range(16):
                    wqkv[m, 2 * hp, rows, :] = lo[hp]
                    wqkv[m, 2 * hp + 1, rows, :] = hi[hp]
        return 0

    jax.lax.fori_loop(0, NT, a_body, 0)

    def g_body(b, _):
        acc = xf[0, b] * gate_ref[0].astype(F32)
        for n in range(1, NT):
            acc = acc + xf[n, b] * gate_ref[n].astype(F32)
        gs = jax.nn.sigmoid(jnp.sum(acc, axis=1, keepdims=True))
        gbuf[b] = jnp.broadcast_to(gs, (128, 128))
        return 0

    jax.lax.fori_loop(0, 16, g_body, 0)
    for n in range(NT):
        wo_copy(n).wait()

    scale = DH ** -0.5
    ri = jax.lax.broadcasted_iota(jnp.int32, (48, 48), 0)
    ci = jax.lax.broadcasted_iota(jnp.int32, (48, 48), 1)
    mask = ((ri < M) | (ri >= ci)) & (ci < M + SEG)

    def wtile(m, hd):
        return pltpu.bitcast(wqkv[m, hd], BF16)

    def attend(q, k, v):
        s = jax.lax.dot_general(q.astype(BF16), k.astype(BF16), (((1,), (1,)), ((), ())),
                                preferred_element_type=F32) * scale
        s = jnp.where(mask, s, -1e9)
        e = jnp.exp(s - jnp.max(s, axis=1, keepdims=True))
        p = e / jnp.sum(e, axis=1, keepdims=True)
        return _dot(p.astype(BF16), v.astype(BF16))

    def project(o_heads, nrows):
        acc = [None] * NT
        for grp in range(H // 4):
            og = jnp.concatenate(o_heads[4 * grp:4 * grp + 4], axis=1).astype(BF16)
            for n in range(NT):
                w = wo_v[n, 4 * grp:4 * grp + 4].reshape(512, 128)
                r = _dot(og, w)
                acc[n] = r if acc[n] is None else acc[n] + r
        return jnp.concatenate(acc, axis=1)

    def o_copy(j, slot):
        return pltpu.make_async_copy(ob.at[slot], out_hbm.at[0, pl.ds(pl.multiple_of(j * 64, 64), 64), :],
                                     sem_o.at[slot])

    def b_body(j, mem):
        b = j // 2
        r0 = pl.multiple_of((j % 2) * 64, 64)

        def xrows(off, n):
            return jnp.concatenate([xf[c, b, pl.ds(r0 + off, n), :] for c in range(NT)], axis=1)

        h = jnp.concatenate([mem, xrows(0, 40)], axis=0).astype(BF16)
        o1 = []
        for hd in range(H):
            q, k, v = _dot(h, wtile(0, hd)), _dot(h, wtile(1, hd)), _dot(h, wtile(2, hd))
            carry[0, hd], carry[1, hd], carry[2, hd] = q[40:48], k[40:48], v[40:48]
            o = attend(q, k, v)
            carry[3, hd] = o[32:40]
            o1.append(o[0:32])
        r1 = project(o1, 32)
        mem = r1[0:8].astype(BF16).astype(F32)
        h = jnp.concatenate([mem, xrows(40, 24)], axis=0).astype(BF16)
        zpad = jnp.zeros((8, 128), F32)
        o2 = []
        for hd in range(H):
            q, k, v = _dot(h, wtile(0, hd)), _dot(h, wtile(1, hd)), _dot(h, wtile(2, hd))
            q = jnp.concatenate([q[0:8], carry[0, hd], q[8:32], zpad], axis=0)
            k = jnp.concatenate([k[0:8], carry[1, hd], k[8:32], zpad], axis=0)
            v = jnp.concatenate([v[0:8], carry[2, hd], v[8:32], zpad], axis=0)
            o = attend(q, k, v)
            o2.append(jnp.concatenate([o[0:8], carry[3, hd], o[8:40]], axis=0))
        r2 = project(o2, 48)
        mem = r2[0:8].astype(BF16).astype(F32)
        bout = jnp.concatenate([r1[8:32], r2[8:48]], axis=0)
        gg = gbuf[b, pl.ds(r0, 64), :]
        slot = j % 2

        @pl.when(j >= 2)
        def _():
            o_copy(j - 2, slot).wait()

        for n in range(NT):
            res = gg * ab[n, b, pl.ds(r0, 64), :] + (1.0 - gg) * bout[:, n * 128:(n + 1) * 128]
            ob[slot, :, n * 128:(n + 1) * 128] = res.astype(BF16)
        o_copy(j, slot).start()
        return mem

    jax.lax.fori_loop(0, NBLK, b_body, mem0_ref[0].astype(F32))
    o_copy(NBLK - 2, 0).wait()
    o_copy(NBLK - 1, 1).wait()


@functools.partial(jax.jit, static_argnames=("B_seg_len",))
def pallas_gated_mix__ssm_conv_h3__memory_aug_recurrent_mem_tr__prompt_kernel(
    A_q, A_k, A_v, A_shift_k, A_ssm_k, A_ssm_D, B_x, B_mem0, B_Wq, B_Wk, B_Wv, B_Wo, B_seg_len, gate_w,
):
    del B_x
    assert int(B_seg_len) == SEG and A_q.shape == (1, S, D) and B_mem0.shape == (1, M, D)
    any_spec = pl.BlockSpec(memory_space=pl.ANY)
    vmem = pl.BlockSpec(memory_space=pltpu.VMEM)
    scratch = [
        pltpu.VMEM((NT, S, 128), BF16),
        pltpu.VMEM((NT, 16, 128, 128), F32),
        pltpu.VMEM((NT, 16, 128, 128), F32),
        pltpu.VMEM((2, S, 128), BF16),
        pltpu.VMEM((2, S, 128), BF16),
        pltpu.VMEM((2, 128, S), BF16),
        pltpu.VMEM((2, 3, CH, H, DH), BF16),
        pltpu.VMEM((3, H, D // 2, 128), jnp.uint32),
        pltpu.VMEM((NT, H, DH, 128), BF16),
        pltpu.VMEM((S + 8, 128), F32),
        pltpu.VMEM((16, 128, 256), F32),
        pltpu.VMEM((32, 128, 256), F32),
        pltpu.VMEM((32, 128, 128), F32),
        pltpu.VMEM((16, 128, 128), F32),
        pltpu.VMEM((4, H, 8, 128), F32),
        pltpu.VMEM((2, 64, D), BF16),
        pltpu.SemaphoreType.DMA((NT,)),
        pltpu.SemaphoreType.DMA((3, 2)),
        pltpu.SemaphoreType.DMA((3, 2)),
        pltpu.SemaphoreType.DMA((NT,)),
        pltpu.SemaphoreType.DMA((2,)),
    ]
    return pl.pallas_call(
        _kernel,
        out_shape=jax.ShapeDtypeStruct((1, S, D), A_q.dtype),
        in_specs=[any_spec] * 8 + [vmem] * 10,
        out_specs=any_spec,
        scratch_shapes=scratch,
        compiler_params=pltpu.CompilerParams(vmem_limit_bytes=120 * 2**20),
    )(A_q, A_k, A_v, A_ssm_k, B_Wq, B_Wk, B_Wv, B_Wo,
      A_shift_k, A_ssm_D.reshape(NT, 1, 128), gate_w.reshape(NT, 1, 128), B_mem0, *_CONSTS)
```

```python
import functools

import jax
import jax.numpy as jnp
import ml_dtypes
import numpy as np
from jax.experimental import pallas as pl
from jax.experimental.pallas import tpu as pltpu

S, D, H, DH, M, SEG = 2048, 1024, 32, 128, 8, 32
NT = D // 128
NBLK = S // (2 * SEG)
CH = 128
F32, BF16 = jnp.float32, jnp.bfloat16


def _make_consts():
    n, tp = 2 * S, 2 * np.pi
    t1 = np.arange(16)
    c1 = np.zeros((16, 256, 128))
    c1i = np.zeros((16, 128, 256))
    for g in range(16):
        for s in range(8):
            t = 128 * t1 + 8 * g + s
            cols = t1 * 8 + s
            c1[g, s, cols] = 1.0
            c1[g, 8 + s, cols] = (-1.0) ** t1
            c1i[g, cols, s] = 1.0 / n
            c1i[g, cols, 8 + s] = (-1.0) ** t1 / n
            for j in range(1, 16):
                ph = tp * ((t * j) % n) / n
                c1[g, 16 * j + s, cols] = np.cos(ph)
                c1[g, 16 * j + 8 + s, cols] = -np.sin(ph)
                c1i[g, cols, 16 * j + s] = 2 * np.cos(ph) / n
                c1i[g, cols, 16 * j + 8 + s] = -2 * np.sin(ph) / n
    a = np.arange(128)
    th = tp * ((a[:, None] * a[None, :]) % 128) / 128
    c, s_ = np.cos(th), np.sin(th)
    th16 = tp * ((a[None, :] * (32 * a[:, None] + 16)) % n) / n
    c2 = np.block([[c, s_], [-s_, c]])
    c2i = np.block([[c, -s_], [s_, c]])
    c2e = np.stack([np.concatenate([c, -s_], 0),
                    np.concatenate([np.cos(th16), -np.sin(th16)], 0)])
    c2ie = np.stack([np.concatenate([c, -s_], 1),
                     np.concatenate([np.cos(th16.T), -np.sin(th16.T)], 1)])
    return tuple(x.astype(ml_dtypes.bfloat16) for x in (c1, c1i, c2, c2i, c2e, c2ie))


_CONSTS = _make_consts()


def _dot(a, b):
    return jnp.dot(a, b, preferred_element_type=F32)


def _kernel(x_hbm, k_hbm, v_hbm, f_hbm, wq_hbm, wk_hbm, wv_hbm, wo_hbm,
            shift_ref, ssmd_ref, gate_ref, mem0_ref,
            c1_ref, c1i_ref, c2_ref, c2i_ref, c2e_ref, c2ie_ref,
            out_hbm,
            xs, xf, ab, ks, vs, fs, wst, wqkv, wos, wo_u, kpad, sig, yb, ub, gbuf, carry, ob,
            sem_x, sem_a, sem_w, sem_wo, sem_o):
    w_hbm = (wq_hbm, wk_hbm, wv_hbm)

    def x_copy(n):
        return pltpu.make_async_copy(x_hbm.at[0, :, pl.ds(n * 128, 128)], xs.at[n], sem_x.at[n])

    def wo_copy(c, slot):
        return pltpu.make_async_copy(wo_hbm.at[pl.ds(c * 4, 4)], wos.at[slot], sem_wo.at[slot])

    def a_copies(dt, slot):
        c0 = pl.multiple_of(dt * 128, 128)
        return (pltpu.make_async_copy(k_hbm.at[0, :, pl.ds(c0, 128)], ks.at[slot], sem_a.at[0, slot]),
                pltpu.make_async_copy(v_hbm.at[0, :, pl.ds(c0, 128)], vs.at[slot], sem_a.at[1, slot]),
                pltpu.make_async_copy(f_hbm.at[pl.ds(c0, 128), :], fs.at[slot], sem_a.at[2, slot]))

    def w_copies(c, slot):
        r0 = pl.multiple_of(c * CH, CH)
        return tuple(pltpu.make_async_copy(w_hbm[m].at[pl.ds(r0, CH)], wst.at[slot, m], sem_w.at[m, slot])
                     for m in range(3))

    for cp in a_copies(0, 0):
        cp.start()
    x_copy(0).start()
    for cp in w_copies(0, 0):
        cp.start()
    for n in range(1, NT):
        x_copy(n).start()
    wo_copy(0, 0).start()
    kpad[0:8, :] = jnp.zeros((8, 128), F32)

    def a_body(dt, _):
        slot = dt % 2
        for cp in a_copies(dt, slot):
            cp.wait()

        @pl.when(dt + 1 < NT)
        def _():
            for cp in a_copies(dt + 1, 1 - slot):
                cp.start()
            for cp in w_copies(dt + 1, 1 - slot):
                cp.start()
            wo_copy(dt + 1, 1 - slot).start()

        c0 = pl.multiple_of(dt * 128, 128)
        sh = jnp.concatenate([shift_ref[pl.ds(c0, 128), :].astype(F32),
                              jnp.zeros((128, 124), F32)], axis=1).T
        taps = [sh[j:j + 1, :] for j in range(4)]
        dvec = ssmd_ref[dt].astype(F32)
        for b in range(16):
            kpad[8 + b * 128:8 + (b + 1) * 128, :] = ks[slot, b * 128:(b + 1) * 128, :].astype(F32)
        for b in range(16):
            kw = kpad[b * 128:b * 128 + 136, :]
            ksh = kw[8:136] * taps[0]
            for j in range(1, 4):
                ksh = ksh + kw[8 - j:136 - j] * taps[j]
            kv = ksh * vs[slot, b * 128:(b + 1) * 128, :].astype(F32)
            sig[b, :, 0:128] = kv.astype(BF16).astype(F32)
            sig[b, :, 128:256] = fs[slot, :, b * 128:(b + 1) * 128].astype(F32).T
        for g in range(16):
            tile = sig[:, 8 * g:8 * g + 8, :].reshape(128, 256).astype(BF16)
            yb[:, 8 * g:8 * g + 8, :] = _dot(c1_ref[g], tile).reshape(32, 8, 256)

        def cmul(z):
            kr, fr, ki, fi = z[0:128, 0:128], z[0:128, 128:256], z[128:256, 0:128], z[128:256, 128:256]
            return jnp.concatenate([kr * fr - ki * fi, kr * fi + ki * fr], axis=0).astype(BF16)

        for e in range(2):
            z = _dot(c2e_ref[e], yb[e].astype(BF16))
            ub[e] = _dot(c2ie_ref[e], cmul(z))
        for j in range(1, 16):
            z = _dot(c2_ref[...], yb[2 * j:2 * j + 2].reshape(256, 256).astype(BF16))
            ub[2 * j:2 * j + 2] = _dot(c2i_ref[...], cmul(z)).reshape(2, 128, 128)
        x_copy(dt).wait()
        for g in range(16):
            tile = ub[:, 8 * g:8 * g + 8, :].reshape(256, 128).astype(BF16)
            y = _dot(c1i_ref[g], tile).reshape(16, 8, 128)
            kv = sig[:, 8 * g:8 * g + 8, 0:128]
            ab[dt, :, 8 * g:8 * g + 8, :] = y + kv * dvec
        for b in range(16):
            xq = xs[dt, b * 128:(b + 1) * 128, :].astype(F32)
            xf[dt, b] = xq
            ab[dt, b] = ab[dt, b] * xq
        for cp in w_copies(dt, slot):
            cp.wait()
        r0 = dt * (CH // 2)
        for m in range(3):
            for b in range(CH // 16):
                u = pltpu.bitcast(wst[slot, m, b * 16:(b + 1) * 16], jnp.uint32).reshape(8, 2, 16, 128)
                ev, od = u[:, 0], u[:, 1]
                lo = jnp.swapaxes((ev & jnp.uint32(0xFFFF)) | (od << 16), 0, 1)
                hi = jnp.swapaxes((ev >> 16) | (od & jnp.uint32(0xFFFF0000)), 0, 1)
                rows = pl.ds(pl.multiple_of(r0 + b * 8, 8), 8)
                for hp in range(16):
                    wqkv[m, 2 * hp, rows, :] = lo[hp]
                    wqkv[m, 2 * hp + 1, rows, :] = hi[hp]
        wo_copy(dt, slot).wait()
        for i in range(4):
            for n in range(NT):
                wo_u[n, dt * 4 + i] = pltpu.bitcast(wos[slot, i, :, n * 128:(n + 1) * 128], jnp.uint32)
        return 0

    jax.lax.fori_loop(0, NT, a_body, 0)

    def g_body(b, _):
        acc = xf[0, b] * gate_ref[0].astype(F32)
        for n in range(1, NT):
            acc = acc + xf[n, b] * gate_ref[n].astype(F32)
        gs = jax.nn.sigmoid(jnp.sum(acc, axis=1, keepdims=True))
        gbuf[b] = jnp.broadcast_to(gs, (128, 128))
        return 0

    jax.lax.fori_loop(0, 16, g_body, 0)

    scale = DH ** -0.5
    ri = jax.lax.broadcasted_iota(jnp.int32, (48, 48), 0)
    ci = jax.lax.broadcasted_iota(jnp.int32, (48, 48), 1)
    mask = ((ri < M) | (ri >= ci)) & (ci < M + SEG)

    def wtile(m, hd):
        return pltpu.bitcast(wqkv[m, hd], BF16)

    def scores(q, k):
        s = jax.lax.dot_general(q, k, (((1,), (1,)), ((), ())), preferred_element_type=F32) * scale
        s = jnp.where(mask, s, -1e9)
        e = jnp.exp(s - jnp.max(s, axis=1, keepdims=True))
        return (e / jnp.sum(e, axis=1, keepdims=True)).astype(BF16)

    def wo_group(grp, og, acc):
        for n in range(NT):
            w = pltpu.bitcast(wo_u[n, 4 * grp:4 * grp + 4].reshape(256, 128), BF16)
            r = _dot(og, w)
            acc[n] = r if acc[n] is None else acc[n] + r

    def segment(h, second):
        zpad = jnp.zeros((8, 128), F32)
        qs, kk, vv, ps, os_ = {}, {}, {}, {}, {}

        def fix(val, idx, hd):
            if not second:
                carry[idx, hd] = val[40:48]
                return val.astype(BF16)
            return jnp.concatenate([val[0:8], carry[idx, hd], val[8:32], zpad], axis=0).astype(BF16)

        def pv(hd):
            o = _dot(ps.pop(hd), vv.pop(hd))
            if not second:
                carry[3, hd] = o[32:40]
                os_[hd] = o[0:32].astype(BF16)
            else:
                os_[hd] = jnp.concatenate([o[0:8], carry[3, hd], o[8:40]], axis=0).astype(BF16)

        def og(grp):
            return jnp.concatenate([os_.pop(4 * grp + i) for i in range(4)], axis=1)

        for hd in range(H):
            qs[hd] = fix(_dot(h, wtile(0, hd)), 0, hd)
            if hd >= 1:
                ps[hd - 1] = scores(qs.pop(hd - 1), kk.pop(hd - 1))
            kk[hd] = fix(_dot(h, wtile(1, hd)), 1, hd)
            vv[hd] = fix(_dot(h, wtile(2, hd)), 2, hd)
            if hd >= 2:
                pv(hd - 2)
        acc = [None] * NT
        ps[H - 1] = scores(qs.pop(H - 1), kk.pop(H - 1))
        wo_group(0, og(0), acc)
        pv(H - 2)
        wo_group(1, og(1), acc)
        wo_group(2, og(2), acc)
        pv(H - 1)
        for grp in range(3, H // 4):
            wo_group(grp, og(grp), acc)
        return jnp.concatenate(acc, axis=1)

    def o_copy(j, slot):
        return pltpu.make_async_copy(ob.at[slot], out_hbm.at[0, pl.ds(pl.multiple_of(j * 64, 64), 64), :],
                                     sem_o.at[slot])

    def b_body(j, mem):
        b = j // 2
        r0 = pl.multiple_of((j % 2) * 64, 64)

        def xrows(off, n):
            return jnp.concatenate([xf[c, b, pl.ds(r0 + off, n), :] for c in range(NT)], axis=1)

        h = jnp.concatenate([mem, xrows(0, 40)], axis=0).astype(BF16)
        r1 = segment(h, False)
        mem = r1[0:8].astype(BF16).astype(F32)
        h = jnp.concatenate([mem, xrows(40, 24)], axis=0).astype(BF16)
        r2 = segment(h, True)
        mem = r2[0:8].astype(BF16).astype(F32)
        bout = jnp.concatenate([r1[8:32], r2[8:48]], axis=0)
        gg = gbuf[b, pl.ds(r0, 64), :]
        slot = j % 2

        @pl.when(j >= 2)
        def _():
            o_copy(j - 2, slot).wait()

        for n in range(NT):
            res = gg * ab[n, b, pl.ds(r0, 64), :] + (1.0 - gg) * bout[:, n * 128:(n + 1) * 128]
            ob[slot, :, n * 128:(n + 1) * 128] = res.astype(BF16)
        o_copy(j, slot).start()
        return mem

    jax.lax.fori_loop(0, NBLK, b_body, mem0_ref[0].astype(F32))
    o_copy(NBLK - 2, 0).wait()
    o_copy(NBLK - 1, 1).wait()


@functools.partial(jax.jit, static_argnames=("B_seg_len",))
def pallas_gated_mix__ssm_conv_h3__memory_aug_recurrent_mem_tr__prompt_kernel(
    A_q, A_k, A_v, A_shift_k, A_ssm_k, A_ssm_D, B_x, B_mem0, B_Wq, B_Wk, B_Wv, B_Wo, B_seg_len, gate_w,
):
    del B_x
    assert int(B_seg_len) == SEG and A_q.shape == (1, S, D) and B_mem0.shape == (1, M, D)
    any_spec = pl.BlockSpec(memory_space=pl.ANY)
    vmem = pl.BlockSpec(memory_space=pltpu.VMEM)
    scratch = [
        pltpu.VMEM((NT, S, 128), BF16),
        pltpu.VMEM((NT, 16, 128, 128), F32),
        pltpu.VMEM((NT, 16, 128, 128), F32),
        pltpu.VMEM((2, S, 128), BF16),
        pltpu.VMEM((2, S, 128), BF16),
        pltpu.VMEM((2, 128, S), BF16),
        pltpu.VMEM((2, 3, CH, H, DH), BF16),
        pltpu.VMEM((3, H, D // 2, 128), jnp.uint32),
        pltpu.VMEM((2, 4, DH, D), BF16),
        pltpu.VMEM((NT, H, DH // 2, 128), jnp.uint32),
        pltpu.VMEM((S + 8, 128), F32),
        pltpu.VMEM((16, 128, 256), F32),
        pltpu.VMEM((32, 128, 256), F32),
        pltpu.VMEM((32, 128, 128), F32),
        pltpu.VMEM((16, 128, 128), F32),
        pltpu.VMEM((4, H, 8, 128), F32),
        pltpu.VMEM((2, 64, D), BF16),
        pltpu.SemaphoreType.DMA((NT,)),
        pltpu.SemaphoreType.DMA((3, 2)),
        pltpu.SemaphoreType.DMA((3, 2)),
        pltpu.SemaphoreType.DMA((2,)),
        pltpu.SemaphoreType.DMA((2,)),
    ]
    return pl.pallas_call(
        _kernel,
        out_shape=jax.ShapeDtypeStruct((1, S, D), A_q.dtype),
        in_specs=[any_spec] * 8 + [vmem] * 10,
        out_specs=any_spec,
        scratch_shapes=scratch,
        compiler_params=pltpu.CompilerParams(vmem_limit_bytes=120 * 2**20),
    )(A_q, A_k, A_v, A_ssm_k, B_Wq, B_Wk, B_Wv, B_Wo,
      A_shift_k, A_ssm_D.reshape(NT, 1, 128), gate_w.reshape(NT, 1, 128), B_mem0, *_CONSTS)
```

```python
import functools

import jax
import jax.numpy as jnp
import ml_dtypes
import numpy as np
from jax.experimental import pallas as pl
from jax.experimental.pallas import tpu as pltpu

S, D, H, DH, M, SEG = 2048, 1024, 32, 128, 8, 32
NT = D // 128
NBLK = S // (2 * SEG)
CH = 128
F32, BF16 = jnp.float32, jnp.bfloat16


def _make_consts():
    n, tp = 2 * S, 2 * np.pi
    t1 = np.arange(16)
    c1 = np.zeros((16, 256, 128))
    c1i = np.zeros((16, 128, 256))
    for g in range(16):
        for s in range(8):
            t = 128 * t1 + 8 * g + s
            cols = t1 * 8 + s
            c1[g, s, cols] = 1.0
            c1[g, 8 + s, cols] = (-1.0) ** t1
            c1i[g, cols, s] = 1.0 / n
            c1i[g, cols, 8 + s] = (-1.0) ** t1 / n
            for j in range(1, 16):
                ph = tp * ((t * j) % n) / n
                c1[g, 16 * j + s, cols] = np.cos(ph)
                c1[g, 16 * j + 8 + s, cols] = -np.sin(ph)
                c1i[g, cols, 16 * j + s] = 2 * np.cos(ph) / n
                c1i[g, cols, 16 * j + 8 + s] = -2 * np.sin(ph) / n
    a = np.arange(128)
    th = tp * ((a[:, None] * a[None, :]) % 128) / 128
    c, s_ = np.cos(th), np.sin(th)
    th16 = tp * ((a[None, :] * (32 * a[:, None] + 16)) % n) / n
    c2 = np.block([[c, s_], [-s_, c]])
    c2i = np.block([[c, -s_], [s_, c]])
    c2e = np.stack([np.concatenate([c, -s_], 0),
                    np.concatenate([np.cos(th16), -np.sin(th16)], 0)])
    c2ie = np.stack([np.concatenate([c, -s_], 1),
                     np.concatenate([np.cos(th16.T), -np.sin(th16.T)], 1)])
    return tuple(x.astype(ml_dtypes.bfloat16) for x in (c1, c1i, c2, c2i, c2e, c2ie))


_CONSTS = _make_consts()


def _dot(a, b):
    return jnp.dot(a, b, preferred_element_type=F32)


def _kernel(x_hbm, k_hbm, v_hbm, f_hbm, wq_hbm, wk_hbm, wv_hbm, wo_hbm,
            shift_ref, ssmd_ref, gate_ref, mem0_ref,
            c1_ref, c1i_ref, c2_ref, c2i_ref, c2e_ref, c2ie_ref,
            out_hbm,
            xs, xf, ab, ks, vs, fs, wst, wqkv, wos, wo_u, kpad, sig, kvb, yb, ub, gbuf, carry, ob,
            sem_x, sem_a, sem_w, sem_wo, sem_o):
    w_hbm = (wq_hbm, wk_hbm, wv_hbm)

    def x_copy(n):
        return pltpu.make_async_copy(x_hbm.at[0, :, pl.ds(n * 128, 128)], xs.at[n], sem_x.at[n])

    def wo_copy(c, slot):
        return pltpu.make_async_copy(wo_hbm.at[pl.ds(c * 4, 4)], wos.at[slot], sem_wo.at[slot])

    def a_copies(dt, slot):
        c0 = pl.multiple_of(dt * 128, 128)
        return (pltpu.make_async_copy(k_hbm.at[0, :, pl.ds(c0, 128)], ks.at[slot], sem_a.at[0, slot]),
                pltpu.make_async_copy(v_hbm.at[0, :, pl.ds(c0, 128)], vs.at[slot], sem_a.at[1, slot]),
                pltpu.make_async_copy(f_hbm.at[pl.ds(c0, 128), :], fs.at[slot], sem_a.at[2, slot]))

    def w_copies(c, slot):
        r0 = pl.multiple_of(c * CH, CH)
        return tuple(pltpu.make_async_copy(w_hbm[m].at[pl.ds(r0, CH)], wst.at[slot, m], sem_w.at[m, slot])
                     for m in range(3))

    for cp in a_copies(0, 0):
        cp.start()
    x_copy(0).start()
    for cp in w_copies(0, 0):
        cp.start()
    for n in range(1, NT):
        x_copy(n).start()
    wo_copy(0, 0).start()
    kpad[0:8, :] = jnp.zeros((8, 128), F32)

    def a_body(dt, _):
        slot = dt % 2
        for cp in a_copies(dt, slot):
            cp.wait()

        @pl.when(dt + 1 < NT)
        def _():
            for cp in a_copies(dt + 1, 1 - slot):
                cp.start()
            for cp in w_copies(dt + 1, 1 - slot):
                cp.start()
            wo_copy(dt + 1, 1 - slot).start()

        c0 = pl.multiple_of(dt * 128, 128)
        sh = jnp.concatenate([shift_ref[pl.ds(c0, 128), :].astype(F32),
                              jnp.zeros((128, 124), F32)], axis=1).T
        taps = [sh[j:j + 1, :] for j in range(4)]
        dvec = ssmd_ref[dt].astype(F32)
        for b in range(16):
            kpad[8 + b * 128:8 + (b + 1) * 128, :] = ks[slot, b * 128:(b + 1) * 128, :].astype(F32)
            sig[b, :, 0:128] = vs[slot, b * 128:(b + 1) * 128, :].astype(F32)
            sig[b, :, 128:256] = fs[slot, :, b * 128:(b + 1) * 128].astype(F32).T
        r0 = dt * (CH // 2)

        def retile_qkv(m, b):
            u = pltpu.bitcast(wst[slot, m, b * 16:(b + 1) * 16], jnp.uint32).reshape(8, 2, 16, 128)
            ev, od = u[:, 0], u[:, 1]
            lo = jnp.swapaxes((ev & jnp.uint32(0xFFFF)) | (od << 16), 0, 1)
            hi = jnp.swapaxes((ev >> 16) | (od & jnp.uint32(0xFFFF0000)), 0, 1)
            rows = pl.ds(pl.multiple_of(r0 + b * 8, 8), 8)
            for hp in range(16):
                wqkv[m, 2 * hp, rows, :] = lo[hp]
                wqkv[m, 2 * hp + 1, rows, :] = hi[hp]

        def retile_o(i):
            for n in range(NT):
                wo_u[n, dt * 4 + i] = pltpu.bitcast(wos[slot, i, :, n * 128:(n + 1) * 128], jnp.uint32)

        for g in range(16):
            kw = jnp.stack([kpad[t * 128 + 8 * g:t * 128 + 8 * g + 16, :] for t in range(16)])
            ksh = kw[:, 8:16] * taps[0]
            for j in range(1, 4):
                ksh = ksh + kw[:, 8 - j:16 - j] * taps[j]
            kv = (ksh * sig[:, 8 * g:8 * g + 8, 0:128]).astype(BF16)
            kvb[:, 8 * g:8 * g + 8, :] = kv.astype(F32)
            ft = sig[:, 8 * g:8 * g + 8, 128:256].reshape(128, 128).astype(BF16)
            tile = jnp.concatenate([kv.astype(F32).reshape(128, 128).astype(BF16), ft], axis=1)
            yb[:, 8 * g:8 * g + 8, :] = _dot(c1_ref[g], tile).reshape(32, 8, 256)

        def cmul(z):
            kr, fr, ki, fi = z[0:128, 0:128], z[0:128, 128:256], z[128:256, 0:128], z[128:256, 128:256]
            return jnp.concatenate([kr * fr - ki * fi, kr * fi + ki * fr], axis=0).astype(BF16)

        def fwd2(j):
            if j < 2:
                return _dot(c2e_ref[j], yb[j].astype(BF16))
            return _dot(c2_ref[...], yb[2 * j - 2:2 * j].reshape(256, 256).astype(BF16))

        def inv2(j, p):
            if j < 2:
                ub[j] = _dot(c2ie_ref[j], p)
            else:
                ub[2 * j - 2:2 * j] = _dot(c2i_ref[...], p).reshape(2, 128, 128)

        z = fwd2(0)
        for j in range(17):
            zn = fwd2(j + 1) if j < 16 else None
            inv2(j, cmul(z))
            z = zn
        x_copy(dt).wait()
        for g in range(16):
            tile = ub[:, 8 * g:8 * g + 8, :].reshape(256, 128).astype(BF16)
            y = _dot(c1i_ref[g], tile).reshape(16, 8, 128)
            if g % 2 == 0:
                xq2 = jnp.stack([xs[dt, t * 128 + 8 * g:t * 128 + 8 * g + 16, :] for t in range(16)]).astype(F32)
                xf[dt, :, 8 * g:8 * g + 16, :] = xq2
            xq = xq2[:, 8 * (g % 2):8 * (g % 2) + 8]
            ab[dt, :, 8 * g:8 * g + 8, :] = (y + kvb[:, 8 * g:8 * g + 8, :] * dvec) * xq
        for cp in w_copies(dt, slot):
            cp.wait()
        wo_copy(dt, slot).wait()
        for m in range(3):
            for b in range(CH // 16):
                retile_qkv(m, b)
        for i in range(4):
            retile_o(i)
        return 0

    jax.lax.fori_loop(0, NT, a_body, 0)

    def g_body(b, _):
        acc = xf[0, b] * gate_ref[0].astype(F32)
        for n in range(1, NT):
            acc = acc + xf[n, b] * gate_ref[n].astype(F32)
        gs = jax.nn.sigmoid(jnp.sum(acc, axis=1, keepdims=True))
        gbuf[b] = jnp.broadcast_to(gs, (128, 128))
        return 0

    jax.lax.fori_loop(0, 16, g_body, 0)

    scale = DH ** -0.5
    ri = jax.lax.broadcasted_iota(jnp.int32, (48, 48), 0)
    ci = jax.lax.broadcasted_iota(jnp.int32, (48, 48), 1)
    mask = ((ri < M) | (ri >= ci)) & (ci < M + SEG)

    def wtile(m, hd):
        return pltpu.bitcast(wqkv[m, hd], BF16)

    def scores(q, k):
        s = jax.lax.dot_general(q, k, (((1,), (1,)), ((), ())), preferred_element_type=F32) * scale
        s = jnp.where(mask, s, -1e9)
        e = jnp.exp(s - jnp.max(s, axis=1, keepdims=True))
        return (e / jnp.sum(e, axis=1, keepdims=True)).astype(BF16)

    def wo_group(grp, og, acc):
        for n in range(NT):
            w = pltpu.bitcast(wo_u[n, 4 * grp:4 * grp + 4].reshape(256, 128), BF16)
            r = _dot(og, w)
            acc[n] = r if acc[n] is None else acc[n] + r

    def segment(h, second):
        zpad = jnp.zeros((8, 128), F32)
        qs, kk, vv, ps, os_ = {}, {}, {}, {}, {}

        def fix(val, idx, hd):
            if not second:
                carry[idx, hd] = val[40:48]
                return val.astype(BF16)
            return jnp.concatenate([val[0:8], carry[idx, hd], val[8:32], zpad], axis=0).astype(BF16)

        def pv(hd):
            o = _dot(ps.pop(hd), vv.pop(hd))
            if not second:
                carry[3, hd] = o[32:40]
                os_[hd] = o[0:32].astype(BF16)
            else:
                os_[hd] = jnp.concatenate([o[0:8], carry[3, hd], o[8:40]], axis=0).astype(BF16)

        def og(grp):
            return jnp.concatenate([os_.pop(4 * grp + i) for i in range(4)], axis=1)

        for hd in range(H):
            qs[hd] = fix(_dot(h, wtile(0, hd)), 0, hd)
            if hd >= 1:
                ps[hd - 1] = scores(qs.pop(hd - 1), kk.pop(hd - 1))
            kk[hd] = fix(_dot(h, wtile(1, hd)), 1, hd)
            vv[hd] = fix(_dot(h, wtile(2, hd)), 2, hd)
            if hd >= 2:
                pv(hd - 2)
        acc = [None] * NT
        ps[H - 1] = scores(qs.pop(H - 1), kk.pop(H - 1))
        wo_group(0, og(0), acc)
        pv(H - 2)
        wo_group(1, og(1), acc)
        wo_group(2, og(2), acc)
        pv(H - 1)
        for grp in range(3, H // 4):
            wo_group(grp, og(grp), acc)
        return jnp.concatenate(acc, axis=1)

    def o_copy(j, slot):
        return pltpu.make_async_copy(ob.at[slot], out_hbm.at[0, pl.ds(pl.multiple_of(j * 64, 64), 64), :],
                                     sem_o.at[slot])

    def b_body(j, mem):
        b = j // 2
        r0 = pl.multiple_of((j % 2) * 64, 64)

        def xrows(off, n):
            return jnp.concatenate([xf[c, b, pl.ds(r0 + off, n), :] for c in range(NT)], axis=1)

        h = jnp.concatenate([mem, xrows(0, 40)], axis=0).astype(BF16)
        r1 = segment(h, False)
        mem = r1[0:8].astype(BF16).astype(F32)
        h = jnp.concatenate([mem, xrows(40, 24)], axis=0).astype(BF16)
        r2 = segment(h, True)
        mem = r2[0:8].astype(BF16).astype(F32)
        bout = jnp.concatenate([r1[8:32], r2[8:48]], axis=0)
        gg = gbuf[b, pl.ds(r0, 64), :]
        slot = j % 2

        @pl.when(j >= 2)
        def _():
            o_copy(j - 2, slot).wait()

        for n in range(NT):
            res = gg * ab[n, b, pl.ds(r0, 64), :] + (1.0 - gg) * bout[:, n * 128:(n + 1) * 128]
            ob[slot, :, n * 128:(n + 1) * 128] = res.astype(BF16)
        o_copy(j, slot).start()
        return mem

    jax.lax.fori_loop(0, NBLK, b_body, mem0_ref[0].astype(F32))
    o_copy(NBLK - 2, 0).wait()
    o_copy(NBLK - 1, 1).wait()


@functools.partial(jax.jit, static_argnames=("B_seg_len",))
def pallas_gated_mix__ssm_conv_h3__memory_aug_recurrent_mem_tr__prompt_kernel(
    A_q, A_k, A_v, A_shift_k, A_ssm_k, A_ssm_D, B_x, B_mem0, B_Wq, B_Wk, B_Wv, B_Wo, B_seg_len, gate_w,
):
    del B_x
    assert int(B_seg_len) == SEG and A_q.shape == (1, S, D) and B_mem0.shape == (1, M, D)
    any_spec = pl.BlockSpec(memory_space=pl.ANY)
    vmem = pl.BlockSpec(memory_space=pltpu.VMEM)
    scratch = [
        pltpu.VMEM((NT, S, 128), BF16),
        pltpu.VMEM((NT, 16, 128, 128), F32),
        pltpu.VMEM((NT, 16, 128, 128), F32),
        pltpu.VMEM((2, S, 128), BF16),
        pltpu.VMEM((2, S, 128), BF16),
        pltpu.VMEM((2, 128, S), BF16),
        pltpu.VMEM((2, 3, CH, H, DH), BF16),
        pltpu.VMEM((3, H, D // 2, 128), jnp.uint32),
        pltpu.VMEM((2, 4, DH, D), BF16),
        pltpu.VMEM((NT, H, DH // 2, 128), jnp.uint32),
        pltpu.VMEM((S + 8, 128), F32),
        pltpu.VMEM((16, 128, 256), F32),
        pltpu.VMEM((16, 128, 128), F32),
        pltpu.VMEM((32, 128, 256), F32),
        pltpu.VMEM((32, 128, 128), F32),
        pltpu.VMEM((16, 128, 128), F32),
        pltpu.VMEM((4, H, 8, 128), F32),
        pltpu.VMEM((2, 64, D), BF16),
        pltpu.SemaphoreType.DMA((NT,)),
        pltpu.SemaphoreType.DMA((3, 2)),
        pltpu.SemaphoreType.DMA((3, 2)),
        pltpu.SemaphoreType.DMA((2,)),
        pltpu.SemaphoreType.DMA((2,)),
    ]
    return pl.pallas_call(
        _kernel,
        out_shape=jax.ShapeDtypeStruct((1, S, D), A_q.dtype),
        in_specs=[any_spec] * 8 + [vmem] * 10,
        out_specs=any_spec,
        scratch_shapes=scratch,
        compiler_params=pltpu.CompilerParams(vmem_limit_bytes=120 * 2**20),
    )(A_q, A_k, A_v, A_ssm_k, B_Wq, B_Wk, B_Wv, B_Wo,
      A_shift_k, A_ssm_D.reshape(NT, 1, 128), gate_w.reshape(NT, 1, 128), B_mem0, *_CONSTS)
```

```python
import functools

import jax
import jax.numpy as jnp
import ml_dtypes
import numpy as np
from jax.experimental import pallas as pl
from jax.experimental.pallas import tpu as pltpu

S, D, H, DH, M, SEG = 2048, 1024, 32, 128, 8, 32
NT = D // 128
NBLK = S // (2 * SEG)
CH = 128
SA, PA, PL = 1, 1, 2
F32, BF16 = jnp.float32, jnp.bfloat16


def _make_consts():
    n, tp = 2 * S, 2 * np.pi
    t1 = np.arange(16)
    c1 = np.zeros((16, 256, 128))
    c1i = np.zeros((16, 128, 256))
    for g in range(16):
        for s in range(8):
            t = 128 * t1 + 8 * g + s
            cols = t1 * 8 + s
            c1[g, s, cols] = 1.0
            c1[g, 8 + s, cols] = (-1.0) ** t1
            c1i[g, cols, s] = 1.0 / n
            c1i[g, cols, 8 + s] = (-1.0) ** t1 / n
            for j in range(1, 16):
                ph = tp * ((t * j) % n) / n
                c1[g, 16 * j + s, cols] = np.cos(ph)
                c1[g, 16 * j + 8 + s, cols] = -np.sin(ph)
                c1i[g, cols, 16 * j + s] = 2 * np.cos(ph) / n
                c1i[g, cols, 16 * j + 8 + s] = -2 * np.sin(ph) / n
    a = np.arange(128)
    th = tp * ((a[:, None] * a[None, :]) % 128) / 128
    c, s_ = np.cos(th), np.sin(th)
    th16 = tp * ((a[None, :] * (32 * a[:, None] + 16)) % n) / n
    c2 = np.block([[c, s_], [-s_, c]])
    c2i = np.block([[c, -s_], [s_, c]])
    c2e = np.stack([np.concatenate([c, -s_], 0),
                    np.concatenate([np.cos(th16), -np.sin(th16)], 0)])
    c2ie = np.stack([np.concatenate([c, -s_], 1),
                     np.concatenate([np.cos(th16.T), -np.sin(th16.T)], 1)])
    return tuple(x.astype(ml_dtypes.bfloat16) for x in (c1, c1i, c2, c2i, c2e, c2ie))


_CONSTS = _make_consts()


def _dot(a, b):
    return jnp.dot(a, b, preferred_element_type=F32)


def _kernel(x_hbm, k_hbm, v_hbm, f_hbm, wq_hbm, wk_hbm, wv_hbm, wo_hbm, c1_hbm, c1i_hbm,
            shift_ref, ssmd_ref, gate_ref, mem0_ref,
            c2_ref, c2i_ref, c2e_ref, c2ie_ref,
            out_hbm,
            c1_ref, c1i_ref, bo, xs, xf, ab, ks, vs, fs, wst, wqkv, wos, wo_u, kpad, sig, kvb, yb, ub, gbuf, carry, ob,
            sem_x, sem_a, sem_w, sem_wo, sem_o, sem_c):
    w_hbm = (wq_hbm, wk_hbm, wv_hbm)

    def x_copy(n):
        return pltpu.make_async_copy(x_hbm.at[0, :, pl.ds(pl.multiple_of(n * 128, 128), 128)], xs.at[n], sem_x.at[n])

    def wo_copy(c, slot):
        return pltpu.make_async_copy(wo_hbm.at[pl.ds(c * 4, 4)], wos.at[slot], sem_wo.at[slot])

    def a_copies(dt, slot):
        c0 = pl.multiple_of(dt * 128, 128)
        return (pltpu.make_async_copy(k_hbm.at[0, :, pl.ds(c0, 128)], ks.at[slot], sem_a.at[0, slot]),
                pltpu.make_async_copy(v_hbm.at[0, :, pl.ds(c0, 128)], vs.at[slot], sem_a.at[1, slot]),
                pltpu.make_async_copy(f_hbm.at[pl.ds(c0, 128), :], fs.at[slot], sem_a.at[2, slot]))

    def w_copies(c, slot):
        r0 = pl.multiple_of(c * CH, CH)
        return tuple(pltpu.make_async_copy(w_hbm[m].at[pl.ds(r0, CH)], wst.at[slot, m], sem_w.at[m, slot])
                     for m in range(3))

    c_copies = (pltpu.make_async_copy(c1_hbm, c1_ref, sem_c.at[0]),
                pltpu.make_async_copy(c1i_hbm, c1i_ref, sem_c.at[1]))
    for cp in a_copies(0, 0):
        cp.start()
    c_copies[0].start()
    kpad[0:8, :] = jnp.zeros((8, 128), F32)

    def a_body(dt, _):
        slot = dt % 2
        for cp in a_copies(dt, slot):
            cp.wait()

        @pl.when(dt == 0)
        def _():
            x_copy(0).start()
            c_copies[1].start()

        for cp in w_copies(dt, slot):
            cp.start()
        wo_copy(dt, slot).start()

        @pl.when(dt + 1 < NT)
        def _():
            for cp in a_copies(dt + 1, 1 - slot):
                cp.start()
            x_copy(dt + 1).start()

        @pl.when(dt == 0)
        def _():
            c_copies[0].wait()

        c0 = pl.multiple_of(dt * 128, 128)
        sh = shift_ref[:, pl.ds(c0, 128)].astype(F32)
        gvec = gate_ref[dt].astype(F32)
        taps = [sh[j:j + 1, :] for j in range(4)]
        dvec = ssmd_ref[dt].astype(F32)
        for b in range(16):
            kpad[8 + b * 128:8 + (b + 1) * 128, :] = ks[slot, b * 128:(b + 1) * 128, :].astype(F32)
            sig[b, :, 0:128] = vs[slot, b * 128:(b + 1) * 128, :].astype(F32)
            sig[b, :, 128:256] = fs[slot, :, b * 128:(b + 1) * 128].astype(F32).T
        r0 = dt * (CH // 2)

        def retile_qkv(m, b):
            u = pltpu.bitcast(wst[slot, m, b * 16:(b + 1) * 16], jnp.uint32).reshape(8, 2, 16, 128)
            ev, od = u[:, 0], u[:, 1]
            lo = jnp.swapaxes((ev & jnp.uint32(0xFFFF)) | (od << 16), 0, 1)
            hi = jnp.swapaxes((ev >> 16) | (od & jnp.uint32(0xFFFF0000)), 0, 1)
            rows = pl.ds(pl.multiple_of(r0 + b * 8, 8), 8)
            for hp in range(16):
                wqkv[m, 2 * hp, rows, :] = lo[hp]
                wqkv[m, 2 * hp + 1, rows, :] = hi[hp]

        def retile_o(i):
            for n in range(NT):
                wo_u[n, dt * 4 + i] = pltpu.bitcast(wos[slot, i, :, n * 128:(n + 1) * 128], jnp.uint32)

        for g in range(16):
            kw = jnp.stack([kpad[t * 128 + 8 * g:t * 128 + 8 * g + 16, :] for t in range(16)])
            ksh = kw[:, 8:16] * taps[0]
            for j in range(1, 4):
                ksh = ksh + kw[:, 8 - j:16 - j] * taps[j]
            kv = (ksh * sig[:, 8 * g:8 * g + 8, 0:128]).astype(BF16)
            kvb[:, 8 * g:8 * g + 8, :] = kv.astype(F32)
            ft = sig[:, 8 * g:8 * g + 8, 128:256].reshape(128, 128).astype(BF16)
            tile = jnp.concatenate([kv.astype(F32).reshape(128, 128).astype(BF16), ft], axis=1)
            yb[:, 8 * g:8 * g + 8, :] = _dot(c1_ref[g], tile).reshape(32, 8, 256)

        def cmul(z):
            kr, fr, ki, fi = z[0:128, 0:128], z[0:128, 128:256], z[128:256, 0:128], z[128:256, 128:256]
            return jnp.concatenate([kr * fr - ki * fi, kr * fi + ki * fr], axis=0).astype(BF16)

        def fwd2(j):
            if j < 2:
                return _dot(c2e_ref[j], yb[j].astype(BF16))
            return _dot(c2_ref[...], yb[2 * j - 2:2 * j].reshape(256, 256).astype(BF16))

        def inv2(j, p):
            if j < 2:
                ub[j] = _dot(c2ie_ref[j], p)
            else:
                ub[2 * j - 2:2 * j] = _dot(c2i_ref[...], p).reshape(2, 128, 128)

        z = fwd2(0)
        for j in range(17):
            zn = fwd2(j + 1) if j < 16 else None
            inv2(j, cmul(z))
            z = zn
        x_copy(dt).wait()

        @pl.when(dt == 0)
        def _():
            c_copies[1].wait()

        for g in range(16):
            tile = ub[:, 8 * g:8 * g + 8, :].reshape(256, 128).astype(BF16)
            y = _dot(c1i_ref[g], tile).reshape(16, 8, 128)
            if g % 2 == 0:
                xq2 = jnp.stack([xs[dt, t * 128 + 8 * g:t * 128 + 8 * g + 16, :] for t in range(16)]).astype(F32)
                xf[dt, :, 8 * g:8 * g + 16, :] = xq2
                gprev = jnp.where(dt == 0, 0.0, gbuf[:, 8 * g:8 * g + 16, :])
                gbuf[:, 8 * g:8 * g + 16, :] = gprev + xq2 * gvec
            xq = xq2[:, 8 * (g % 2):8 * (g % 2) + 8]
            ab[dt, :, 8 * g:8 * g + 8, :] = (y + kvb[:, 8 * g:8 * g + 8, :] * dvec) * xq
        for cp in w_copies(dt, slot):
            cp.wait()
        wo_copy(dt, slot).wait()
        for m in range(3):
            for b in range(CH // 16):
                retile_qkv(m, b)
        for i in range(4):
            retile_o(i)
        return 0

    jax.lax.fori_loop(0, NT, a_body, 0)

    bo[...] = jnp.zeros(bo.shape, F32)

    scale = DH ** -0.5
    ri = jax.lax.broadcasted_iota(jnp.int32, (80, 96), 0)
    ci = jax.lax.broadcasted_iota(jnp.int32, (80, 96), 1)
    rq, ck = ri % 40, ci % 48
    mask = ((ri >= 40) == (ci >= 48)) & ((rq < M) | (rq >= ck)) & (ck < M + SEG)

    def wtile(m, hd):
        return pltpu.bitcast(wqkv[m, hd], BF16)

    def scores(q2, k2):
        s = jax.lax.dot_general(q2, k2, (((1,), (1,)), ((), ())), preferred_element_type=F32) * scale
        s = jnp.where(mask, s, -1e9)
        e = jnp.exp(s - jnp.max(s, axis=1, keepdims=True))
        return (e / jnp.sum(e, axis=1, keepdims=True)).astype(BF16)

    def wo_group(grp, og, acc):
        for n in range(NT):
            w = pltpu.bitcast(wo_u[n, 4 * grp:4 * grp + 4].reshape(256, 128), BF16)
            r = _dot(og, w)
            acc[n] = r if acc[n] is None else acc[n] + r

    def segment(h, second):
        zpad = jnp.zeros((8, 128), F32)
        qs, kk, vv, ps, os_ = {}, {}, {}, {}, {}

        def fix(val, idx, hd, pad):
            if not second:
                carry[idx, hd] = val[40:48]
                rows = [val[0:40]]
            else:
                rows = [val[0:8], carry[idx, hd], val[8:32]]
            return jnp.concatenate(rows + ([zpad] if pad else []), axis=0)

        def sc(pr):
            q2 = jnp.concatenate([qs.pop(2 * pr), qs.pop(2 * pr + 1)], axis=0).astype(BF16)
            k2 = jnp.concatenate([kk.pop(2 * pr), kk.pop(2 * pr + 1)], axis=0)
            ps[pr] = scores(q2, k2)

        def pv(pr):
            v2 = jnp.concatenate([vv.pop(2 * pr), vv.pop(2 * pr + 1)], axis=0)
            o2 = _dot(ps.pop(pr), v2)
            for i in range(2):
                hd, o = 2 * pr + i, o2[40 * i:40 * i + 40]
                if not second:
                    carry[3, hd] = o[32:40]
                    os_[hd] = o[0:32].astype(BF16)
                else:
                    os_[hd] = jnp.concatenate([o[0:8], carry[3, hd], o[8:40]], axis=0).astype(BF16)

        def og(grp):
            return jnp.concatenate([os_.pop(4 * grp + i) for i in range(4)], axis=1)

        NP = H // 2
        for hd in range(H):
            pr, odd = hd // 2, hd % 2
            qs[hd] = fix(_dot(h, wtile(0, hd)), 0, hd, False)
            if odd == SA and pr >= 1:
                sc(pr - 1)
            kk[hd] = fix(_dot(h, wtile(1, hd)), 1, hd, True).astype(BF16)
            vv[hd] = fix(_dot(h, wtile(2, hd)), 2, hd, True).astype(BF16)
            if odd == PA and pr >= PL:
                pv(pr - PL)
        acc = [None] * NT
        grp = 0
        sc(NP - 1)
        for pr in range(NP - PL, NP):
            wo_group(grp, og(grp), acc)
            wo_group(grp + 1, og(grp + 1), acc)
            grp += 2
            pv(pr)
        for g2 in range(grp, H // 4):
            wo_group(g2, og(g2), acc)
        return jnp.concatenate(acc, axis=1)

    def o_copy(j, slot):
        return pltpu.make_async_copy(ob.at[slot], out_hbm.at[0, pl.ds(pl.multiple_of(j * 64, 64), 64), :],
                                     sem_o.at[slot])

    def epilogue(j):
        b = j // 2
        r0 = pl.multiple_of((j % 2) * 64, 64)
        gg = jax.nn.sigmoid(jnp.sum(gbuf[b, pl.ds(r0, 64), :], axis=1, keepdims=True))
        for n in range(NT):
            res = gg * ab[n, b, pl.ds(r0, 64), :] + (1.0 - gg) * bo[:, n * 128:(n + 1) * 128]
            ob[j % 2, :, n * 128:(n + 1) * 128] = res.astype(BF16)

    def b_body(j, mem):
        b = j // 2
        r0 = pl.multiple_of((j % 2) * 64, 64)

        @pl.when(j >= 3)
        def _():
            o_copy(j - 3, (j - 3) % 2).wait()

        def xrows(off, n):
            return jnp.concatenate([xf[c, b, pl.ds(r0 + off, n), :] for c in range(NT)], axis=1)

        epilogue(jnp.maximum(j - 1, 0))
        h = jnp.concatenate([mem, xrows(0, 40)], axis=0).astype(BF16)
        r1 = segment(h, False)
        mem = r1[0:8].astype(BF16).astype(F32)
        bo[0:24, :] = r1[8:32]
        h = jnp.concatenate([mem, xrows(40, 24)], axis=0).astype(BF16)
        r2 = segment(h, True)
        mem = r2[0:8].astype(BF16).astype(F32)
        bo[24:64, :] = r2[8:48]

        @pl.when(j >= 1)
        def _():
            o_copy(j - 1, (j - 1) % 2).start()

        return mem

    jax.lax.fori_loop(0, NBLK, b_body, mem0_ref[0].astype(F32))
    o_copy(NBLK - 3, (NBLK - 3) % 2).wait()
    epilogue(NBLK - 1)
    o_copy(NBLK - 1, (NBLK - 1) % 2).start()
    o_copy(NBLK - 2, (NBLK - 2) % 2).wait()
    o_copy(NBLK - 1, (NBLK - 1) % 2).wait()


@functools.partial(jax.jit, static_argnames=("B_seg_len",))
def pallas_gated_mix__ssm_conv_h3__memory_aug_recurrent_mem_tr__prompt_kernel(
    A_q, A_k, A_v, A_shift_k, A_ssm_k, A_ssm_D, B_x, B_mem0, B_Wq, B_Wk, B_Wv, B_Wo, B_seg_len, gate_w,
):
    del B_x
    assert int(B_seg_len) == SEG and A_q.shape == (1, S, D) and B_mem0.shape == (1, M, D)
    any_spec = pl.BlockSpec(memory_space=pl.ANY)
    vmem = pl.BlockSpec(memory_space=pltpu.VMEM)
    scratch = [
        pltpu.VMEM((16, 256, 128), BF16),
        pltpu.VMEM((16, 128, 256), BF16),
        pltpu.VMEM((64, D), F32),
        pltpu.VMEM((NT, S, 128), BF16),
        pltpu.VMEM((NT, 16, 128, 128), F32),
        pltpu.VMEM((NT, 16, 128, 128), F32),
        pltpu.VMEM((2, S, 128), BF16),
        pltpu.VMEM((2, S, 128), BF16),
        pltpu.VMEM((2, 128, S), BF16),
        pltpu.VMEM((2, 3, CH, H, DH), BF16),
        pltpu.VMEM((3, H, D // 2, 128), jnp.uint32),
        pltpu.VMEM((2, 4, DH, D), BF16),
        pltpu.VMEM((NT, H, DH // 2, 128), jnp.uint32),
        pltpu.VMEM((S + 8, 128), F32),
        pltpu.VMEM((16, 128, 256), F32),
        pltpu.VMEM((16, 128, 128), F32),
        pltpu.VMEM((32, 128, 256), F32),
        pltpu.VMEM((32, 128, 128), F32),
        pltpu.VMEM((16, 128, 128), F32),
        pltpu.VMEM((4, H, 8, 128), F32),
        pltpu.VMEM((2, 64, D), BF16),
        pltpu.SemaphoreType.DMA((NT,)),
        pltpu.SemaphoreType.DMA((3, 2)),
        pltpu.SemaphoreType.DMA((3, 2)),
        pltpu.SemaphoreType.DMA((2,)),
        pltpu.SemaphoreType.DMA((2,)),
        pltpu.SemaphoreType.DMA((2,)),
    ]
    return pl.pallas_call(
        _kernel,
        out_shape=jax.ShapeDtypeStruct((1, S, D), A_q.dtype),
        in_specs=[any_spec] * 10 + [vmem] * 8,
        out_specs=any_spec,
        scratch_shapes=scratch,
        compiler_params=pltpu.CompilerParams(vmem_limit_bytes=120 * 2**20),
    )(A_q, A_k, A_v, A_ssm_k, B_Wq, B_Wk, B_Wv, B_Wo, _CONSTS[0], _CONSTS[1],
      A_shift_k.T, A_ssm_D.reshape(NT, 1, 128), gate_w.reshape(NT, 1, 128), B_mem0, *_CONSTS[2:])
```

```python
import functools

import jax
import jax.numpy as jnp
import ml_dtypes
import numpy as np
from jax.experimental import pallas as pl
from jax.experimental.pallas import tpu as pltpu

S, D, H, DH, M, SEG = 2048, 1024, 32, 128, 8, 32
NT = D // 128
NBLK = S // (2 * SEG)
CH = 128
SA, PA, PL = 1, 1, 2
F32, BF16 = jnp.float32, jnp.bfloat16


def _make_consts():
    n, tp = 2 * S, 2 * np.pi
    t1 = np.arange(16)
    c1 = np.zeros((16, 256, 128))
    c1i = np.zeros((16, 128, 256))
    for g in range(16):
        for s in range(8):
            t = 128 * t1 + 8 * g + s
            cols = t1 * 8 + s
            c1[g, s, cols] = 1.0
            c1[g, 8 + s, cols] = (-1.0) ** t1
            c1i[g, cols, s] = 1.0 / n
            c1i[g, cols, 8 + s] = (-1.0) ** t1 / n
            for j in range(1, 16):
                ph = tp * ((t * j) % n) / n
                c1[g, 16 * j + s, cols] = np.cos(ph)
                c1[g, 16 * j + 8 + s, cols] = -np.sin(ph)
                c1i[g, cols, 16 * j + s] = 2 * np.cos(ph) / n
                c1i[g, cols, 16 * j + 8 + s] = -2 * np.sin(ph) / n
    a = np.arange(128)
    th = tp * ((a[:, None] * a[None, :]) % 128) / 128
    c, s_ = np.cos(th), np.sin(th)
    th16 = tp * ((a[None, :] * (32 * a[:, None] + 16)) % n) / n
    c2 = np.block([[c, s_], [-s_, c]])
    c2i = np.block([[c, -s_], [s_, c]])
    c2e = np.stack([np.concatenate([c, -s_], 0),
                    np.concatenate([np.cos(th16), -np.sin(th16)], 0)])
    c2ie = np.stack([np.concatenate([c, -s_], 1),
                     np.concatenate([np.cos(th16.T), -np.sin(th16.T)], 1)])
    return tuple(x.astype(ml_dtypes.bfloat16) for x in (c1, c1i, c2, c2i, c2e, c2ie))


_CONSTS = _make_consts()


def _dot(a, b):
    return jnp.dot(a, b, preferred_element_type=F32)


def _transpose8(x):
    sub = jax.lax.broadcasted_iota(jnp.int32, (8, 128), 0)
    x = list(x)
    for s in (4, 2, 1):
        keep = (sub & s) == 0
        for j in range(8):
            if j & s == 0:
                a, b = x[j], x[j + s]
                x[j] = jnp.where(keep, a, pltpu.roll(b, s, 0))
                x[j + s] = jnp.where(keep, pltpu.roll(a, 8 - s, 0), b)
    return x


def _kernel(x_hbm, k_hbm, v_hbm, f_hbm, wq_hbm, wk_hbm, wv_hbm, wo_hbm, c1_hbm, c1i_hbm,
            shift_ref, ssmd_ref, gate_ref, mem0_ref,
            c2_ref, c2i_ref, c2e_ref, c2ie_ref,
            out_hbm,
            c1_ref, c1i_ref, bo, xs, xf, ab, ks, vs, fs, wst, wqkv, wos, wo_u, kpad, sig, kvb, yb, ub, gbuf, carry, ob,
            sem_x, sem_a, sem_w, sem_wo, sem_o, sem_c):
    w_hbm = (wq_hbm, wk_hbm, wv_hbm)

    def x_copy(n):
        return pltpu.make_async_copy(x_hbm.at[0, :, pl.ds(pl.multiple_of(n * 128, 128), 128)], xs.at[n], sem_x.at[n])

    def wo_copy(c, slot):
        return pltpu.make_async_copy(wo_hbm.at[pl.ds(c * 4, 4)], wos.at[slot], sem_wo.at[slot])

    def a_copies(dt, slot):
        c0 = pl.multiple_of(dt * 128, 128)
        return (pltpu.make_async_copy(k_hbm.at[0, :, pl.ds(c0, 128)], ks.at[slot], sem_a.at[0, slot]),
                pltpu.make_async_copy(v_hbm.at[0, :, pl.ds(c0, 128)], vs.at[slot], sem_a.at[1, slot]),
                pltpu.make_async_copy(f_hbm.at[pl.ds(c0, 128), :], fs.at[slot], sem_a.at[2, slot]))

    def w_copies(c, slot):
        r0 = pl.multiple_of(c * CH, CH)
        return tuple(pltpu.make_async_copy(w_hbm[m].at[pl.ds(r0, CH)], wst.at[slot, m], sem_w.at[m, slot])
                     for m in range(3))

    c_copies = (pltpu.make_async_copy(c1_hbm, c1_ref, sem_c.at[0]),
                pltpu.make_async_copy(c1i_hbm, c1i_ref, sem_c.at[1]))
    for cp in a_copies(0, 0):
        cp.start()
    c_copies[0].start()
    kpad[0:8, :] = jnp.zeros((8, 128), F32)

    def a_body(dt, _):
        slot = dt % 2
        for cp in a_copies(dt, slot):
            cp.wait()

        @pl.when(dt == 0)
        def _():
            x_copy(0).start()
            c_copies[1].start()

        for cp in w_copies(dt, slot):
            cp.start()
        wo_copy(dt, slot).start()

        @pl.when(dt + 1 < NT)
        def _():
            for cp in a_copies(dt + 1, 1 - slot):
                cp.start()
            x_copy(dt + 1).start()

        @pl.when(dt == 0)
        def _():
            c_copies[0].wait()

        c0 = pl.multiple_of(dt * 128, 128)
        sh = shift_ref[:, pl.ds(c0, 128)].astype(F32)
        gvec = gate_ref[dt].astype(F32)
        taps = [sh[j:j + 1, :] for j in range(4)]
        dvec = ssmd_ref[dt].astype(F32)
        for b in range(16):
            kpad[8 + b * 128:8 + (b + 1) * 128, :] = ks[slot, b * 128:(b + 1) * 128, :].astype(F32)
            sig[b, :, 0:128] = vs[slot, b * 128:(b + 1) * 128, :].astype(F32)
            sig[b, :, 128:256] = fs[slot, :, b * 128:(b + 1) * 128].astype(F32).T
        r0 = dt * (CH // 2)

        def retile_qkv(m, b):
            u = pltpu.bitcast(wst[slot, m, b * 16:(b + 1) * 16], jnp.uint32).reshape(8, 2, 16, 128)
            ev, od = u[:, 0], u[:, 1]
            lo = (ev & jnp.uint32(0xFFFF)) | (od << 16)
            hi = (ev >> 16) | (od & jnp.uint32(0xFFFF0000))
            rows = pl.ds(pl.multiple_of(r0 + b * 8, 8), 8)
            for par, val in enumerate((lo, hi)):
                for half in range(2):
                    t = _transpose8([val[i, 8 * half:8 * half + 8] for i in range(8)])
                    for i in range(8):
                        wqkv[m, 2 * (8 * half + i) + par, rows, :] = t[i]

        def retile_o(i):
            for n in range(NT):
                wo_u[n, dt * 4 + i] = pltpu.bitcast(wos[slot, i, :, n * 128:(n + 1) * 128], jnp.uint32)

        for g in range(16):
            kw = jnp.stack([kpad[t * 128 + 8 * g:t * 128 + 8 * g + 16, :] for t in range(16)])
            ksh = kw[:, 8:16] * taps[0]
            for j in range(1, 4):
                ksh = ksh + kw[:, 8 - j:16 - j] * taps[j]
            kv = (ksh * sig[:, 8 * g:8 * g + 8, 0:128]).astype(BF16)
            kvb[:, 8 * g:8 * g + 8, :] = kv.astype(F32)
            ft = sig[:, 8 * g:8 * g + 8, 128:256].reshape(128, 128).astype(BF16)
            tile = jnp.concatenate([kv.astype(F32).reshape(128, 128).astype(BF16), ft], axis=1)
            yb[:, 8 * g:8 * g + 8, :] = _dot(c1_ref[g], tile).reshape(32, 8, 256)

        def cmul(z):
            kr, fr, ki, fi = z[0:128, 0:128], z[0:128, 128:256], z[128:256, 0:128], z[128:256, 128:256]
            return jnp.concatenate([kr * fr - ki * fi, kr * fi + ki * fr], axis=0).astype(BF16)

        def fwd2(j):
            if j < 2:
                return _dot(c2e_ref[j], yb[j].astype(BF16))
            return _dot(c2_ref[...], yb[2 * j - 2:2 * j].reshape(256, 256).astype(BF16))

        def inv2(j, p):
            if j < 2:
                ub[j] = _dot(c2ie_ref[j], p)
            else:
                ub[2 * j - 2:2 * j] = _dot(c2i_ref[...], p).reshape(2, 128, 128)

        z = fwd2(0)
        for j in range(17):
            zn = fwd2(j + 1) if j < 16 else None
            inv2(j, cmul(z))
            z = zn
        x_copy(dt).wait()

        @pl.when(dt == 0)
        def _():
            c_copies[1].wait()

        for g in range(16):
            tile = ub[:, 8 * g:8 * g + 8, :].reshape(256, 128).astype(BF16)
            y = _dot(c1i_ref[g], tile).reshape(16, 8, 128)
            if g % 2 == 0:
                xq2 = jnp.stack([xs[dt, t * 128 + 8 * g:t * 128 + 8 * g + 16, :] for t in range(16)]).astype(F32)
                xf[dt, :, 8 * g:8 * g + 16, :] = xq2
                gprev = jnp.where(dt == 0, 0.0, gbuf[:, 8 * g:8 * g + 16, :])
                gbuf[:, 8 * g:8 * g + 16, :] = gprev + xq2 * gvec
            xq = xq2[:, 8 * (g % 2):8 * (g % 2) + 8]
            ab[dt, :, 8 * g:8 * g + 8, :] = (y + kvb[:, 8 * g:8 * g + 8, :] * dvec) * xq
        for cp in w_copies(dt, slot):
            cp.wait()
        wo_copy(dt, slot).wait()
        for m in range(3):
            for b in range(CH // 16):
                retile_qkv(m, b)
        for i in range(4):
            retile_o(i)
        return 0

    jax.lax.fori_loop(0, NT, a_body, 0)

    bo[...] = jnp.zeros(bo.shape, F32)

    scale = DH ** -0.5
    ri = jax.lax.broadcasted_iota(jnp.int32, (80, 96), 0)
    ci = jax.lax.broadcasted_iota(jnp.int32, (80, 96), 1)
    rq, ck = ri % 40, ci % 48
    mask = ((ri >= 40) == (ci >= 48)) & ((rq < M) | (rq >= ck)) & (ck < M + SEG)

    def wtile(m, hd):
        return pltpu.bitcast(wqkv[m, hd], BF16)

    def scores(q2, k2):
        s = jax.lax.dot_general(q2, k2, (((1,), (1,)), ((), ())), preferred_element_type=F32) * scale
        s = jnp.where(mask, s, -1e9)
        e = jnp.exp(s - jnp.max(s, axis=1, keepdims=True))
        return (e / jnp.sum(e, axis=1, keepdims=True)).astype(BF16)

    def wo_group(grp, og, acc):
        for n in range(NT):
            w = pltpu.bitcast(wo_u[n, 4 * grp:4 * grp + 4].reshape(256, 128), BF16)
            r = _dot(og, w)
            acc[n] = r if acc[n] is None else acc[n] + r

    def segment(h, second):
        zpad = jnp.zeros((8, 128), F32)
        qs, kk, vv, ps, os_ = {}, {}, {}, {}, {}

        def fix(val, idx, hd, pad):
            if not second:
                carry[idx, hd] = val[40:48]
                rows = [val[0:40]]
            else:
                rows = [val[0:8], carry[idx, hd], val[8:32]]
            return jnp.concatenate(rows + ([zpad] if pad else []), axis=0)

        def sc(pr):
            q2 = jnp.concatenate([qs.pop(2 * pr), qs.pop(2 * pr + 1)], axis=0).astype(BF16)
            k2 = jnp.concatenate([kk.pop(2 * pr), kk.pop(2 * pr + 1)], axis=0)
            ps[pr] = scores(q2, k2)

        def pv(pr):
            v2 = jnp.concatenate([vv.pop(2 * pr), vv.pop(2 * pr + 1)], axis=0)
            o2 = _dot(ps.pop(pr), v2)
            for i in range(2):
                hd, o = 2 * pr + i, o2[40 * i:40 * i + 40]
                if not second:
                    carry[3, hd] = o[32:40]
                    os_[hd] = o[0:32].astype(BF16)
                else:
                    os_[hd] = jnp.concatenate([o[0:8], carry[3, hd], o[8:40]], axis=0).astype(BF16)

        def og(grp):
            return jnp.concatenate([os_.pop(4 * grp + i) for i in range(4)], axis=1)

        NP = H // 2
        for hd in range(H):
            pr, odd = hd // 2, hd % 2
            qs[hd] = fix(_dot(h, wtile(0, hd)), 0, hd, False)
            if odd == SA and pr >= 1:
                sc(pr - 1)
            kk[hd] = fix(_dot(h, wtile(1, hd)), 1, hd, True).astype(BF16)
            vv[hd] = fix(_dot(h, wtile(2, hd)), 2, hd, True).astype(BF16)
            if odd == PA and pr >= PL:
                pv(pr - PL)
        acc = [None] * NT
        grp = 0
        sc(NP - 1)
        for pr in range(NP - PL, NP):
            wo_group(grp, og(grp), acc)
            wo_group(grp + 1, og(grp + 1), acc)
            grp += 2
            pv(pr)
        for g2 in range(grp, H // 4):
            wo_group(g2, og(g2), acc)
        return jnp.concatenate(acc, axis=1)

    def o_copy(j, slot):
        return pltpu.make_async_copy(ob.at[slot], out_hbm.at[0, pl.ds(pl.multiple_of(j * 64, 64), 64), :],
                                     sem_o.at[slot])

    def epilogue(j):
        b = j // 2
        r0 = pl.multiple_of((j % 2) * 64, 64)
        gg = jax.nn.sigmoid(jnp.sum(gbuf[b, pl.ds(r0, 64), :], axis=1, keepdims=True))
        for n in range(NT):
            res = gg * ab[n, b, pl.ds(r0, 64), :] + (1.0 - gg) * bo[:, n * 128:(n + 1) * 128]
            ob[j % 2, :, n * 128:(n + 1) * 128] = res.astype(BF16)

    def b_body(j, mem):
        b = j // 2
        r0 = pl.multiple_of((j % 2) * 64, 64)

        @pl.when(j >= 3)
        def _():
            o_copy(j - 3, (j - 3) % 2).wait()

        def xrows(off, n):
            return jnp.concatenate([xf[c, b, pl.ds(r0 + off, n), :] for c in range(NT)], axis=1)

        epilogue(jnp.maximum(j - 1, 0))
        h = jnp.concatenate([mem, xrows(0, 40)], axis=0).astype(BF16)
        r1 = segment(h, False)
        mem = r1[0:8].astype(BF16).astype(F32)
        bo[0:24, :] = r1[8:32]
        h = jnp.concatenate([mem, xrows(40, 24)], axis=0).astype(BF16)
        r2 = segment(h, True)
        mem = r2[0:8].astype(BF16).astype(F32)
        bo[24:64, :] = r2[8:48]

        @pl.when(j >= 1)
        def _():
            o_copy(j - 1, (j - 1) % 2).start()

        return mem

    jax.lax.fori_loop(0, NBLK, b_body, mem0_ref[0].astype(F32))
    o_copy(NBLK - 3, (NBLK - 3) % 2).wait()
    epilogue(NBLK - 1)
    o_copy(NBLK - 1, (NBLK - 1) % 2).start()
    o_copy(NBLK - 2, (NBLK - 2) % 2).wait()
    o_copy(NBLK - 1, (NBLK - 1) % 2).wait()


@functools.partial(jax.jit, static_argnames=("B_seg_len",))
def pallas_gated_mix__ssm_conv_h3__memory_aug_recurrent_mem_tr__prompt_kernel(
    A_q, A_k, A_v, A_shift_k, A_ssm_k, A_ssm_D, B_x, B_mem0, B_Wq, B_Wk, B_Wv, B_Wo, B_seg_len, gate_w,
):
    del B_x
    assert int(B_seg_len) == SEG and A_q.shape == (1, S, D) and B_mem0.shape == (1, M, D)
    any_spec = pl.BlockSpec(memory_space=pl.ANY)
    vmem = pl.BlockSpec(memory_space=pltpu.VMEM)
    scratch = [
        pltpu.VMEM((16, 256, 128), BF16),
        pltpu.VMEM((16, 128, 256), BF16),
        pltpu.VMEM((64, D), F32),
        pltpu.VMEM((NT, S, 128), BF16),
        pltpu.VMEM((NT, 16, 128, 128), F32),
        pltpu.VMEM((NT, 16, 128, 128), F32),
        pltpu.VMEM((2, S, 128), BF16),
        pltpu.VMEM((2, S, 128), BF16),
        pltpu.VMEM((2, 128, S), BF16),
        pltpu.VMEM((2, 3, CH, H, DH), BF16),
        pltpu.VMEM((3, H, D // 2, 128), jnp.uint32),
        pltpu.VMEM((2, 4, DH, D), BF16),
        pltpu.VMEM((NT, H, DH // 2, 128), jnp.uint32),
        pltpu.VMEM((S + 8, 128), F32),
        pltpu.VMEM((16, 128, 256), F32),
        pltpu.VMEM((16, 128, 128), F32),
        pltpu.VMEM((32, 128, 256), F32),
        pltpu.VMEM((32, 128, 128), F32),
        pltpu.VMEM((16, 128, 128), F32),
        pltpu.VMEM((4, H, 8, 128), F32),
        pltpu.VMEM((2, 64, D), BF16),
        pltpu.SemaphoreType.DMA((NT,)),
        pltpu.SemaphoreType.DMA((3, 2)),
        pltpu.SemaphoreType.DMA((3, 2)),
        pltpu.SemaphoreType.DMA((2,)),
        pltpu.SemaphoreType.DMA((2,)),
        pltpu.SemaphoreType.DMA((2,)),
    ]
    return pl.pallas_call(
        _kernel,
        out_shape=jax.ShapeDtypeStruct((1, S, D), A_q.dtype),
        in_specs=[any_spec] * 10 + [vmem] * 8,
        out_specs=any_spec,
        scratch_shapes=scratch,
        compiler_params=pltpu.CompilerParams(vmem_limit_bytes=120 * 2**20),
    )(A_q, A_k, A_v, A_ssm_k, B_Wq, B_Wk, B_Wv, B_Wo, _CONSTS[0], _CONSTS[1],
      A_shift_k.T, A_ssm_D.reshape(NT, 1, 128), gate_w.reshape(NT, 1, 128), B_mem0, *_CONSTS[2:])
```

```python
import functools

import jax
import jax.numpy as jnp
import ml_dtypes
import numpy as np
from jax.experimental import pallas as pl
from jax.experimental.pallas import tpu as pltpu

S, D, H, DH, M, SEG = 2048, 1024, 32, 128, 8, 32
NT = D // 128
NBLK = S // (2 * SEG)
CH = 128
GS, GD = 4, 2
SA, PA, PL = 1, 1, 2
F32, BF16 = jnp.float32, jnp.bfloat16


def _make_consts():
    n, tp = 2 * S, 2 * np.pi
    t1 = np.arange(16)
    c1 = np.zeros((16, 256, 128))
    c1i = np.zeros((16, 128, 256))
    for g in range(16):
        for s in range(8):
            t = 128 * t1 + 8 * g + s
            cols = t1 * 8 + s
            c1[g, s, cols] = 1.0
            c1[g, 8 + s, cols] = (-1.0) ** t1
            c1i[g, cols, s] = 1.0 / n
            c1i[g, cols, 8 + s] = (-1.0) ** t1 / n
            for j in range(1, 16):
                ph = tp * ((t * j) % n) / n
                c1[g, 16 * j + s, cols] = np.cos(ph)
                c1[g, 16 * j + 8 + s, cols] = -np.sin(ph)
                c1i[g, cols, 16 * j + s] = 2 * np.cos(ph) / n
                c1i[g, cols, 16 * j + 8 + s] = -2 * np.sin(ph) / n
    a = np.arange(128)
    th = tp * ((a[:, None] * a[None, :]) % 128) / 128
    c, s_ = np.cos(th), np.sin(th)
    th16 = tp * ((a[None, :] * (32 * a[:, None] + 16)) % n) / n
    c2 = np.block([[c, s_], [-s_, c]])
    c2i = np.block([[c, -s_], [s_, c]])
    c2e = np.stack([np.concatenate([c, -s_], 0),
                    np.concatenate([np.cos(th16), -np.sin(th16)], 0)])
    c2ie = np.stack([np.concatenate([c, -s_], 1),
                     np.concatenate([np.cos(th16.T), -np.sin(th16.T)], 1)])
    return tuple(x.astype(ml_dtypes.bfloat16) for x in (c1, c1i, c2, c2i, c2e, c2ie))


_CONSTS = _make_consts()


def _dot(a, b):
    return jnp.dot(a, b, preferred_element_type=F32)


def _transpose8(x):
    sub = jax.lax.broadcasted_iota(jnp.int32, (8, 128), 0)
    x = list(x)
    for s in (4, 2, 1):
        keep = (sub & s) == 0
        for j in range(8):
            if j & s == 0:
                a, b = x[j], x[j + s]
                x[j] = jnp.where(keep, a, pltpu.roll(b, s, 0))
                x[j + s] = jnp.where(keep, pltpu.roll(a, 8 - s, 0), b)
    return x


def _kernel(x_hbm, k_hbm, v_hbm, f_hbm, wq_hbm, wk_hbm, wv_hbm, wo_hbm, c1_hbm, c1i_hbm,
            shift_ref, ssmd_ref, gate_ref, mem0_ref,
            c2_ref, c2i_ref, c2e_ref, c2ie_ref,
            out_hbm,
            c1_ref, c1i_ref, bo, xs, xf, ab, ks, vs, fs, wst, wqkv, wos, wo_u, kpad, sig, kvb, yb, ub, gbuf, carry, ob,
            sem_x, sem_a, sem_w, sem_wo, sem_o, sem_c):
    w_hbm = (wq_hbm, wk_hbm, wv_hbm)

    def x_copy(n):
        return pltpu.make_async_copy(x_hbm.at[0, :, pl.ds(pl.multiple_of(n * 128, 128), 128)], xs.at[n], sem_x.at[n])

    def wo_copy(c, slot):
        return pltpu.make_async_copy(wo_hbm.at[pl.ds(c * 4, 4)], wos.at[slot], sem_wo.at[slot])

    def a_copies(dt, slot):
        c0 = pl.multiple_of(dt * 128, 128)
        return (pltpu.make_async_copy(k_hbm.at[0, :, pl.ds(c0, 128)], ks.at[slot], sem_a.at[0, slot]),
                pltpu.make_async_copy(v_hbm.at[0, :, pl.ds(c0, 128)], vs.at[slot], sem_a.at[1, slot]),
                pltpu.make_async_copy(f_hbm.at[pl.ds(c0, 128), :], fs.at[slot], sem_a.at[2, slot]))

    def w_copies(c, slot):
        r0 = pl.multiple_of(c * CH, CH)
        return tuple(pltpu.make_async_copy(w_hbm[m].at[pl.ds(r0, CH)], wst.at[slot, m], sem_w.at[m, slot])
                     for m in range(3))

    c_copies = (pltpu.make_async_copy(c1_hbm, c1_ref, sem_c.at[0]),
                pltpu.make_async_copy(c1i_hbm, c1i_ref, sem_c.at[1]))
    for cp in a_copies(0, 0):
        cp.start()
    c_copies[0].start()
    kpad[0:8, :] = jnp.zeros((8, 128), F32)

    def a_body(dt, _):
        slot = dt % 2
        for cp in a_copies(dt, slot):
            cp.wait()

        @pl.when(dt == 0)
        def _():
            x_copy(0).start()
            c_copies[1].start()

        for cp in w_copies(dt, slot):
            cp.start()
        wo_copy(dt, slot).start()

        @pl.when(dt + 1 < NT)
        def _():
            for cp in a_copies(dt + 1, 1 - slot):
                cp.start()
            x_copy(dt + 1).start()

        @pl.when(dt == 0)
        def _():
            c_copies[0].wait()

        c0 = pl.multiple_of(dt * 128, 128)
        sh = shift_ref[:, pl.ds(c0, 128)].astype(F32)
        gvec = gate_ref[dt].astype(F32)
        taps = [sh[j:j + 1, :] for j in range(4)]
        dvec = ssmd_ref[dt].astype(F32)
        for b in range(16):
            kpad[8 + b * 128:8 + (b + 1) * 128, :] = ks[slot, b * 128:(b + 1) * 128, :].astype(F32)
            sig[b, :, 0:128] = vs[slot, b * 128:(b + 1) * 128, :].astype(F32)
            sig[b, :, 128:256] = fs[slot, :, b * 128:(b + 1) * 128].astype(F32).T
        r0 = dt * (CH // 2)

        def retile_qkv(m, b):
            u = pltpu.bitcast(wst[slot, m, b * 16:(b + 1) * 16], jnp.uint32).reshape(8, 2, 16, 128)
            ev, od = u[:, 0], u[:, 1]
            lo = (ev & jnp.uint32(0xFFFF)) | (od << 16)
            hi = (ev >> 16) | (od & jnp.uint32(0xFFFF0000))
            rows = pl.ds(pl.multiple_of(r0 + b * 8, 8), 8)
            for par, val in enumerate((lo, hi)):
                for half in range(2):
                    t = _transpose8([val[i, 8 * half:8 * half + 8] for i in range(8)])
                    for i in range(8):
                        wqkv[m, 2 * (8 * half + i) + par, rows, :] = t[i]

        def retile_o(i):
            for n in range(NT):
                wo_u[n, dt * 4 + i] = pltpu.bitcast(wos[slot, i, :, n * 128:(n + 1) * 128], jnp.uint32)

        for g in range(16):
            kw = jnp.stack([kpad[t * 128 + 8 * g:t * 128 + 8 * g + 16, :] for t in range(16)])
            ksh = kw[:, 8:16] * taps[0]
            for j in range(1, 4):
                ksh = ksh + kw[:, 8 - j:16 - j] * taps[j]
            kv = (ksh * sig[:, 8 * g:8 * g + 8, 0:128]).astype(BF16)
            kvb[:, 8 * g:8 * g + 8, :] = kv.astype(F32)
            ft = sig[:, 8 * g:8 * g + 8, 128:256].reshape(128, 128).astype(BF16)
            tile = jnp.concatenate([kv.astype(F32).reshape(128, 128).astype(BF16), ft], axis=1)
            r = _dot(c1_ref[g], tile).reshape(32, 8, 256)
            if g % 2 == 0:
                r_even = r
            else:
                yb[:, 8 * g - 8:8 * g + 8, :] = jnp.concatenate([r_even, r], axis=1).astype(BF16)

        def cmul(z):
            kr, fr, ki, fi = z[0:128, 0:128], z[0:128, 128:256], z[128:256, 0:128], z[128:256, 128:256]
            return jnp.concatenate([kr * fr - ki * fi, kr * fi + ki * fr], axis=0).astype(BF16)

        def fwd2(j):
            if j < 2:
                return _dot(c2e_ref[j], yb[j])
            return _dot(c2_ref[...], yb[2 * j - 2:2 * j].reshape(256, 256))

        def inv2(j, p):
            if j < 2:
                ub[j] = _dot(c2ie_ref[j], p)
            else:
                ub[2 * j - 2:2 * j] = _dot(c2i_ref[...], p).reshape(2, 128, 128)

        z = fwd2(0)
        for j in range(17):
            zn = fwd2(j + 1) if j < 16 else None
            inv2(j, cmul(z))
            z = zn
        x_copy(dt).wait()

        @pl.when(dt == 0)
        def _():
            c_copies[1].wait()

        for g in range(16):
            tile = ub[:, 8 * g:8 * g + 8, :].reshape(256, 128).astype(BF16)
            y = _dot(c1i_ref[g], tile).reshape(16, 8, 128)
            if g % 2 == 0:
                xq2 = jnp.stack([xs[dt, t * 128 + 8 * g:t * 128 + 8 * g + 16, :] for t in range(16)]).astype(F32)
                xf[dt, :, 8 * g:8 * g + 16, :] = xq2
                gprev = jnp.where(dt == 0, 0.0, gbuf[:, 8 * g:8 * g + 16, :])
                gbuf[:, 8 * g:8 * g + 16, :] = gprev + xq2 * gvec
            xq = xq2[:, 8 * (g % 2):8 * (g % 2) + 8]
            ab[dt, :, 8 * g:8 * g + 8, :] = (y + kvb[:, 8 * g:8 * g + 8, :] * dvec) * xq
        for cp in w_copies(dt, slot):
            cp.wait()
        wo_copy(dt, slot).wait()
        for m in range(3):
            for b in range(CH // 16):
                retile_qkv(m, b)
        for i in range(4):
            retile_o(i)
        return 0

    jax.lax.fori_loop(0, NT, a_body, 0)

    bo[...] = jnp.zeros(bo.shape, F32)

    scale = DH ** -0.5
    ri = jax.lax.broadcasted_iota(jnp.int32, (80, 96), 0)
    ci = jax.lax.broadcasted_iota(jnp.int32, (80, 96), 1)
    rq, ck = ri % 40, ci % 48
    real = ((ri >= 40) == (ci >= 48)) & (ck < M + SEG)
    mask = real & ((rq < M) | (rq >= ck))
    fill = jnp.where(real, -1e9, -jnp.inf)

    def wtile(m, hd):
        return pltpu.bitcast(wqkv[m, hd], BF16)

    def scores(q2, k2):
        s = jax.lax.dot_general(q2, k2, (((1,), (1,)), ((), ())), preferred_element_type=F32) * scale
        s = jnp.where(mask, s, fill)
        e = jnp.exp(s - jnp.max(s, axis=1, keepdims=True))
        return (e / jnp.sum(e, axis=1, keepdims=True)).astype(BF16)

    def wo_group(grp, og, acc):
        for n in range(NT):
            w = pltpu.bitcast(wo_u[n, GS * grp:GS * grp + GS].reshape(GS * 64, 128), BF16)
            r = _dot(og, w)
            acc[n] = r if acc[n] is None else acc[n] + r

    def segment(h, second):
        zpad = jnp.zeros((8, 128), F32)
        qs, kk, vv, ps, os_ = {}, {}, {}, {}, {}

        def fix(val, idx, hd, pad):
            if not second:
                carry[idx, hd] = val[40:48]
                rows = [val[0:40]]
            else:
                rows = [val[0:8], carry[idx, hd], val[8:32]]
            return jnp.concatenate(rows + ([zpad] if pad else []), axis=0)

        def sc(pr):
            q2 = jnp.concatenate([qs.pop(2 * pr), qs.pop(2 * pr + 1)], axis=0).astype(BF16)
            k2 = jnp.concatenate([kk.pop(2 * pr), kk.pop(2 * pr + 1)], axis=0)
            ps[pr] = scores(q2, k2)

        def pv(pr):
            v2 = jnp.concatenate([vv.pop(2 * pr), vv.pop(2 * pr + 1)], axis=0)
            o2 = _dot(ps.pop(pr), v2)
            for i in range(2):
                hd, o = 2 * pr + i, o2[40 * i:40 * i + 40]
                if not second:
                    carry[3, hd] = o[32:40]
                    os_[hd] = o[0:32].astype(BF16)
                else:
                    os_[hd] = jnp.concatenate([o[0:8], carry[3, hd], o[8:40]], axis=0).astype(BF16)

        def og(grp):
            return jnp.concatenate([os_.pop(GS * grp + i) for i in range(GS)], axis=1)

        NP = H // 2
        for hd in range(H):
            pr, odd = hd // 2, hd % 2
            qs[hd] = fix(_dot(h, wtile(0, hd)), 0, hd, False)
            if odd == SA and pr >= 1:
                sc(pr - 1)
            kk[hd] = fix(_dot(h, wtile(1, hd)), 1, hd, True).astype(BF16)
            vv[hd] = fix(_dot(h, wtile(2, hd)), 2, hd, True).astype(BF16)
            if odd == PA and pr >= PL:
                pv(pr - PL)
        acc = [None] * NT
        grp = 0
        sc(NP - 1)
        for pr in range(NP - PL, NP):
            for _ in range(GD):
                wo_group(grp, og(grp), acc)
                grp += 1
            pv(pr)
        for g2 in range(grp, H // GS):
            wo_group(g2, og(g2), acc)
        return jnp.concatenate(acc, axis=1)

    def o_copy(j):
        return pltpu.make_async_copy(ob.at[j], out_hbm.at[0, pl.ds(pl.multiple_of(j * 64, 64), 64), :],
                                     sem_o.at[0])

    def epilogue(j):
        b = j // 2
        r0 = pl.multiple_of((j % 2) * 64, 64)
        gg = jax.nn.sigmoid(jnp.sum(gbuf[b, pl.ds(r0, 64), :], axis=1, keepdims=True))
        for n in range(NT):
            res = gg * ab[n, b, pl.ds(r0, 64), :] + (1.0 - gg) * bo[:, n * 128:(n + 1) * 128]
            ob[j, :, n * 128:(n + 1) * 128] = res.astype(BF16)

    def b_body(j, mem):
        b = j // 2
        r0 = pl.multiple_of((j % 2) * 64, 64)

        def xrows(off, n):
            return jnp.concatenate([xf[c, b, pl.ds(r0 + off, n), :] for c in range(NT)], axis=1)

        epilogue(jnp.maximum(j - 1, 0))
        h = jnp.concatenate([mem, xrows(0, 40)], axis=0).astype(BF16)
        r1 = segment(h, False)
        mem = r1[0:8]
        bo[0:24, :] = r1[8:32]
        h = jnp.concatenate([mem, xrows(40, 24)], axis=0).astype(BF16)
        r2 = segment(h, True)
        mem = r2[0:8]
        bo[24:64, :] = r2[8:48]

        @pl.when(j >= 1)
        def _():
            o_copy(j - 1).start()

        return mem

    jax.lax.fori_loop(0, NBLK, b_body, mem0_ref[0].astype(F32), unroll=2)
    epilogue(NBLK - 1)
    o_copy(NBLK - 1).start()
    for j in range(NBLK):
        o_copy(j).wait()


@functools.partial(jax.jit, static_argnames=("B_seg_len",))
def pallas_gated_mix__ssm_conv_h3__memory_aug_recurrent_mem_tr__prompt_kernel(
    A_q, A_k, A_v, A_shift_k, A_ssm_k, A_ssm_D, B_x, B_mem0, B_Wq, B_Wk, B_Wv, B_Wo, B_seg_len, gate_w,
):
    del B_x
    assert int(B_seg_len) == SEG and A_q.shape == (1, S, D) and B_mem0.shape == (1, M, D)
    any_spec = pl.BlockSpec(memory_space=pl.ANY)
    vmem = pl.BlockSpec(memory_space=pltpu.VMEM)
    scratch = [
        pltpu.VMEM((16, 256, 128), BF16),
        pltpu.VMEM((16, 128, 256), BF16),
        pltpu.VMEM((64, D), F32),
        pltpu.VMEM((NT, S, 128), BF16),
        pltpu.VMEM((NT, 16, 128, 128), F32),
        pltpu.VMEM((NT, 16, 128, 128), F32),
        pltpu.VMEM((2, S, 128), BF16),
        pltpu.VMEM((2, S, 128), BF16),
        pltpu.VMEM((2, 128, S), BF16),
        pltpu.VMEM((2, 3, CH, H, DH), BF16),
        pltpu.VMEM((3, H, D // 2, 128), jnp.uint32),
        pltpu.VMEM((2, 4, DH, D), BF16),
        pltpu.VMEM((NT, H, DH // 2, 128), jnp.uint32),
        pltpu.VMEM((S + 8, 128), F32),
        pltpu.VMEM((16, 128, 256), F32),
        pltpu.VMEM((16, 128, 128), F32),
        pltpu.VMEM((32, 128, 256), BF16),
        pltpu.VMEM((32, 128, 128), F32),
        pltpu.VMEM((16, 128, 128), F32),
        pltpu.VMEM((4, H, 8, 128), F32),
        pltpu.VMEM((NBLK, 64, D), BF16),
        pltpu.SemaphoreType.DMA((NT,)),
        pltpu.SemaphoreType.DMA((3, 2)),
        pltpu.SemaphoreType.DMA((3, 2)),
        pltpu.SemaphoreType.DMA((2,)),
        pltpu.SemaphoreType.DMA((2,)),
        pltpu.SemaphoreType.DMA((2,)),
    ]
    return pl.pallas_call(
        _kernel,
        out_shape=jax.ShapeDtypeStruct((1, S, D), A_q.dtype),
        in_specs=[any_spec] * 10 + [vmem] * 8,
        out_specs=any_spec,
        scratch_shapes=scratch,
        compiler_params=pltpu.CompilerParams(vmem_limit_bytes=120 * 2**20),
    )(A_q, A_k, A_v, A_ssm_k, B_Wq, B_Wk, B_Wv, B_Wo, _CONSTS[0], _CONSTS[1],
      A_shift_k.T, A_ssm_D.reshape(NT, 1, 128), gate_w.reshape(NT, 1, 128), B_mem0, *_CONSTS[2:])
```
